```python
import os as _os
_os.environ.setdefault("JAX_PLATFORMS", "cpu")
import jax
import jax.numpy as jnp

def _softmax(x, axis=-1):
    return jax.nn.softmax(x, axis=axis)
def _gelu(x):
    return jax.nn.gelu(x, approximate=True)
def _silu(x):
    return jax.nn.silu(x)
def _sigmoid(x):
    return jax.nn.sigmoid(x)
def _layernorm(x, axis=-1, eps=1e-5):
    m = jnp.mean(x, axis=axis, keepdims=True)
    v = jnp.var(x, axis=axis, keepdims=True)
    return (x - m) / jnp.sqrt(v + eps)
def _scatter_add(tgt, idx, src, axis=0):
    return tgt.at[idx].add(src)
def _segment_sum(src, seg, n):
    return jax.ops.segment_sum(src, seg, n)
class _Rng:
    def __init__(self, key):
        self._k = key
    def _next(self):
        self._k, sub = jax.random.split(self._k)
        return sub
    def normal(self, shape):
        return jax.random.normal(self._next(), shape, dtype=jnp.bfloat16)
    def randint(self, lo, hi, shape):
        return jax.random.randint(self._next(), shape, lo, hi, dtype=jnp.int32)
    def uniform(self, shape, lo=0.0, hi=1.0):
        return jax.random.uniform(self._next(), shape, jnp.bfloat16, lo, hi)
    def permutation(self, n):
        return jax.random.permutation(self._next(), n)


kernel_name = 'gated_mix__ssm_conv_h3__mixer_s_mlp__prompt'

def setup_inputs():
    _rng = _Rng(jax.random.key(int.from_bytes(__import__("os").urandom(4), "little")))
    _w = (lambda a: (lambda t: t.astype(jnp.bfloat16) if jnp.issubdtype(t.dtype, jnp.floating) else t)(jnp.asarray(a)))
    def _A_setup():
        B, S, D = 1, 2048, 576
        ks = 4
        return {
            "q": _w((lambda *s: _rng.normal(s) * 0.05)(B, S, D)),
            "k": _w((lambda *s: _rng.normal(s) * 0.4)(B, S, D)),
            "v": _w((lambda *s: _rng.normal(s) * 0.4)(B, S, D)),
            "shift_k": _w((lambda *s: _rng.normal(s) * 0.4)(D, ks) * 0.5),
            "ssm_k": _w((lambda *s: _rng.normal(s) * 0.4)(D, S) * (1.0 / S ** 0.5)),
            "ssm_D": _w((lambda *s: _rng.normal(s) * 0.4)(D)),
        }
    _A_in = _A_setup()

    def _B_setup():
        B, S, D, F = 1, 2048, 576, 4608
        return {
            "x":  _w((lambda *s: _rng.normal(s) * 0.05)(B, S, D)),
            "w1": _w((lambda *s: _rng.normal(s) * 0.2)(D, D) * (D ** -0.5)),
            "w2": _w((lambda *s: _rng.normal(s) * 0.2)(D, D) * (D ** -0.5)),
            "w3": _w((lambda *s: _rng.normal(s) * 0.2)(D, F) * (D ** -0.5)),
            "w4": _w((lambda *s: _rng.normal(s) * 0.2)(F, D) * (F ** -0.5)),
        }
    _B_in = _B_setup()

    return {
        "A_q": _A_in["q"],
        "A_k": _A_in["k"],
        "A_v": _A_in["v"],
        "A_shift_k": _A_in["shift_k"],
        "A_ssm_k": _A_in["ssm_k"],
        "A_ssm_D": _A_in["ssm_D"],
        "B_x": _B_in["x"],
        "B_w1": _B_in["w1"],
        "B_w2": _B_in["w2"],
        "B_w3": _B_in["w3"],
        "B_w4": _B_in["w4"],
        "gate_w": _w((lambda *s: _rng.normal(s) * 0.05)(576) * 16.0),
    }

def reference(A_q, A_k, A_v, A_shift_k, A_ssm_k, A_ssm_D, B_x, B_w1, B_w2, B_w3, B_w4, gate_w):
    def _A_ref(q, k, v, shift_k, ssm_k, ssm_D):
        B, S, D = q.shape
        ks = shift_k.shape[-1]
        k_pad = jnp.pad(k, ((0, 0), (ks - 1, 0), (0, 0)))
        k_shift = jnp.zeros_like(k)
        for t in range(ks):
            k_shift = k_shift + k_pad[:, t:t + S, :] * shift_k[:, ks - 1 - t][None, None, :]
        kv = k_shift * v
        L = 2 * S
        kv_pad = jnp.pad(kv, ((0, 0), (0, S), (0, 0)))
        kf_pad = jnp.pad(ssm_k, ((0, 0), (0, S)))
        kv_f = (lambda x, axes=(-2,-1): jnp.fft.rfft2(x.astype(jnp.float32), axes=axes))(kv_pad[:, None, :, :], axes=(1, 2))
        kf_f = (lambda x, axes=(-2,-1): jnp.fft.rfft2(x.astype(jnp.float32), axes=axes))(kf_pad[:, None, :], axes=(1, 2))
        kf_f = (lambda x, *d: x.transpose(*d))(kf_f, 1, 2, 0)
        y_f = kv_f * kf_f[None, :, :, :]
        y = (lambda x, s, axes=(-2,-1): jnp.fft.irfft2(x, s=s, axes=axes).astype(jnp.bfloat16))(y_f, (1, L), axes=(1, 2))[:, 0, :S, :]
        y = y + kv * ssm_D[None, None, :]
        return q * y

    def _B_ref(x, w1, w2, w3, w4):
        B, S, D = x.shape
        h = _gelu(_layernorm(x, axis=-1) @ w1)
        c = D // 4
        g0 = jnp.pad(h[:, :, 0*c:1*c], ((0, 0), (1, 0), (0, 0)))[:, :S, :]
        g1 = jnp.pad(h[:, :, 1*c:2*c], ((0, 0), (0, 1), (0, 0)))[:, 1:, :]
        g2 = jnp.pad(h[:, :, 2*c:3*c], ((0, 0), (2, 0), (0, 0)))[:, :S, :]
        g3 = jnp.pad(h[:, :, 3*c:   ], ((0, 0), (0, 2), (0, 0)))[:, 2:, :]
        hs = jnp.concatenate([g0, g1, g2, g3], axis=-1) @ w2
        x1 = x + hs
        h2 = _gelu(_layernorm(x1, axis=-1) @ w3) @ w4
        return x1 + h2

    x = A_q
    g = _sigmoid((x * gate_w).sum(-1, keepdims=True))
    a = _A_ref(x, A_k, A_v, A_shift_k, A_ssm_k, A_ssm_D)
    b = _B_ref(x, B_w1, B_w2, B_w3, B_w4)
    return g * a + (1 - g) * b
```

```python
import numpy as np
import ml_dtypes
import jax
import jax.numpy as jnp
from jax import lax
import jax.experimental.pallas as pl
import jax.experimental.pallas.tpu as pltpu

S, D, F = 2048, 576, 4608
T = 128
NTILE = S // T
RG = D // 16
KT = 3
FC = 4 * KT * T
NFC = F // FC
NTG = NTILE // 4
NU = NFC * NTG
CG = RG // NU
DQ = D // 4
EPS = 1e-5
GC0 = float(np.sqrt(2.0 / np.pi))
ALPHA = float((0.044715 * GC0) ** (1.0 / 3.0))
f32 = jnp.float32
bf16 = jnp.bfloat16
u32 = jnp.uint32
NT_DIMS = (((1,), (1,)), ((), ()))

A_TAB = (((1, 0), (1, 3)), ((1, 2), (1, 3)), ((1, 0),), ((1, 3),), ((1, 0), (1, 1)), ((1, 2), (-1, 0)), ((1, 1), (-1, 3)))
B_TAB = (((1, 0), (1, 3)), ((1, 0),), ((1, 1), (-1, 3)), ((1, 2), (-1, 0)), ((1, 3),), ((1, 0), (1, 1)), ((1, 2), (1, 3)))
C_TAB = (((1, 0), (1, 3)), ((1, 2), (-1, 3)), ((1, 1), (1, 3)), ((1, 0), (1, 2)), ((-1, 0), (1, 1)), ((1, 3),), ((1, 0),))
E_TAB = (None, ((1, 2),), ((1, 1),), None, None, ((1, 3), (-1, 1), (1, 2)), ((1, 0),))
R_TAB = (None, (1, 0), None, None, (0, 1), (1, 2), (0, 2))
BLANK = [7 * _i + _j for _i in range(7) for _j in range(7) if E_TAB[_i] is None or E_TAB[_j] is None]


def _dft_mats():
    n = np.arange(T, dtype=np.float64)[:, None]
    f = np.arange(T, dtype=np.float64)[None, :]
    th = 2.0 * np.pi * (f + 0.5) * n / (2 * T)
    fwd = np.concatenate([np.cos(th), -np.sin(th)], axis=1)
    inv = fwd.T / T
    fwd = np.stack([fwd[:, :T], fwd[:, T:]])
    return fwd.astype(ml_dtypes.bfloat16), inv[None].astype(ml_dtypes.bfloat16)


def _comb(tab, q):
    (_, a), *rest = tab
    v = q[a]
    for s, b in rest:
        v = v + q[b] if s > 0 else v - q[b]
    return v


def _ccomb(m):
    return [m[0] + m[3] - m[4] + m[6], m[2] + m[4], m[1] + m[3], m[0] - m[1] + m[2] + m[5]]


def _blk(o, p):
    return 2 * (o // 2) + p // 2, 2 * (o % 2) + p % 2


def _gelu(h):
    return h * (1.0 + jnp.tanh(h * (GC0 / ALPHA + h * h)))


def _interleave(*streams):
    st = []
    for s in streams:
        lo, hi = (s[2], s[3]) if len(s) > 2 else (0.0, 1.0)
        st.append([0.0, float(s[0]) or 1.0, s[1], lo, hi])
    while st:
        st.sort(key=lambda x: x[3] + (x[4] - x[3]) * x[0] / x[1])
        try:
            st[0][0] += next(st[0][2])
        except StopIteration:
            st.pop(0)


def _chain(*streams):
    def g():
        for s in streams:
            yield from s[1]
    return sum(s[0] for s in streams), g()


def _run(*streams):
    for s in streams:
        for _ in s[1]:
            pass


import contextlib


def make(prof=0, pp=24, gst=0, nb=2, gauss=0, ska=0.98, skb=0.87, sk1=0.9, esplit=25, upto=99, pz=0, pb=0, px=0, pw=2, pa=0, py=0, skf=0.9, only=None, e2=0, pv=3, p4=0, s0=0, wr=13, wg=30, wc=35, ca=0, wl=32):
    scope = jax.named_scope if prof else (lambda n: contextlib.nullcontext())

    def kernel(q_hbm, k_hbm, v_hbm, sk_hbm, f_hbm, d_hbm, w1_hbm, w2_hbm, w3_hbm, w4_hbm, gw_hbm, fwd_hbm, inv_hbm,
               out_hbm,
               q_v, k_v, v_v, f_v, w1_v, w2_v, w3_v, w4_v, sk_v, d_v, gw_v, fwd_v, inv_v,
               w1t, w2t, coef, sign, g_v, XN0, XN1, HR, X1a, X1b, X1c, X1d, XT, XS, XE, WR, W3C, W4C, P0, P1, B, B2, acc,
               KV, Z, Y, ga, o_v, zs, sems, osems, bsems):
        P = (P0, P1)
        XN = (XN0, XN1)
        X1 = (X1a, X1b, X1c, X1d)

        def packed(ref, idx):
            v = ref.bitcast(u32)[idx]
            if v.ndim == 3:
                v = v.reshape(v.shape[0] * v.shape[1], v.shape[2])
            return pltpu.bitcast(v, bf16)

        pairs = dict(gw=(gw_hbm, gw_v), sk=(sk_hbm, sk_v), d=(d_hbm, d_v), w1=(w1_hbm, w1_v), w2=(w2_hbm, w2_v),
                     fwd=(fwd_hbm, fwd_v), inv=(inv_hbm, inv_v))

        def part(name, src, dst, idx):
            pairs[name] = (src.at[idx], dst.at[idx])

        every = slice(None)
        for g in range(NTG):
            part('q%d' % g, q_hbm, q_v, (every, every, pl.ds(g * 4 * T, 4 * T)))
        for n, src_, dst_, first in (('k', k_hbm, k_v, 3 * CG), ('v', v_hbm, v_v, 3 * CG), ('f', f_hbm, f_v, 2 * CG)):
            part(n + '0', src_, dst_, pl.ds(0, first))
            part(n, src_, dst_, pl.ds(first, RG - first))
        for fq in range(4):
            part('w3_a%d' % fq, w3_hbm, w3_v, (every, every, pl.ds(fq * KT * T, T)))
            part('w3_b%d' % fq, w3_hbm, w3_v, (every, every, pl.ds(fq * KT * T + T, (KT - 1) * T)))
        for t in range(NFC):
            if t:
                part('w3_%d' % t, w3_hbm, w3_v, (every, every, pl.ds(t * FC, FC)))
            part('w4_%d' % t, w4_hbm, w4_v, (every, every, pl.ds(t * FC, FC)))
        w3_a, w3_b = (['w3_%s%d' % (ab, fq) for fq in range(4)] for ab in 'ab')
        names = ['gw', 'sk', 'd', 'q0', 'w1', 'q1', 'w2', 'q2', 'q3'] + w3_a + ['k0', 'v0'] + w3_b \
            + ['w4_0', 'f0', 'fwd', 'inv', 'w3_1', 'f', 'k', 'v', 'w4_1', 'w3_2', 'w4_2']
        cp = {n: pltpu.make_async_copy(pairs[n][0], pairs[n][1], sems.at[i]) for i, n in enumerate(names)}

        def start(*ns):
            for n in ns:
                cp[n].start()

        def wait(*ns):
            with scope('wait_' + '_'.join(ns)):
                for n in ns:
                    cp[n].wait()

        start(*names)
        for i in range(16):
            zs[i] = 0
        HR[0] = jnp.zeros((D, T), bf16)
        HR[NTILE + 1] = jnp.zeros((D, T), bf16)
        sign[...] = (1 - 2 * (lax.broadcasted_iota(jnp.int32, (16, T), 1) & 1)).astype(f32)
        zero = []

        def load_zeros():
            zero[:] = [zs[i] for i in range(16)]

        lane16 = lax.broadcasted_iota(jnp.int32, (16, T), 1)
        lane72 = lax.broadcasted_iota(jnp.int32, (DQ // 2, T), 1)

        def combos16(tab, blk, store):
            for i in range(7):
                inner = [_comb(tab[i], [blk[_blk(o, p)[0]][_blk(o, p)[1]] for o in range(4)]) for p in range(4)]
                for j in range(7):
                    store(7 * i + j, _comb(tab[j], inner).astype(bf16))
                yield wc

        def recombine8(load):
            h = [[None] * 4 for _ in range(4)]
            for i in range(7):
                q = _ccomb([load(7 * i + j) for j in range(7)])
                for s, o in C_TAB[i]:
                    for p in range(4):
                        a, b = _blk(o, p)
                        if h[a][b] is None:
                            h[a][b] = q[p] if s > 0 else -q[p]
                        else:
                            h[a][b] = h[a][b] + q[p] if s > 0 else h[a][b] - q[p]
                yield wr
            return h

        def transpose_w(src, dst):
            def g():
                for kt in range(5):
                    n = T if kt < 4 else D - 4 * T
                    w = src[kt * T:kt * T + n, :].astype(f32)
                    if n < T:
                        w = jnp.concatenate([w, jnp.zeros((T - n, D), f32)], axis=0)
                    dst[kt] = w.T.astype(bf16)
                    yield 100
            return 500, g()

        def coefs(which):
            def g():
                for i in which:
                    if i < 4:
                        r = sk_v[...].astype(f32)[i:i + 1]
                    else:
                        r = (d_v if i == 4 else gw_v)[...].astype(f32).reshape(1, D)
                    coef[i] = jnp.broadcast_to(r, (T, D)).T.reshape(RG, 16, T)
                    yield 80
            return 80 * len(which), g()

        def vsum(x):
            parts = [x[r:r + 8] for r in range(0, x.shape[0], 8)]
            while len(parts) > 1:
                parts = [parts[i] + parts[i + 1] for i in range(0, len(parts) - 1, 2)] + ([parts[-1]] if len(parts) % 2 else [])
            return parts[0]

        def rows8(stat, n):
            return jnp.concatenate([stat] * (n // 8), axis=0)

        def centred_scale(xg, ca, sm, z):
            mean = jnp.broadcast_to(jnp.sum(sm, axis=0, keepdims=True) * (1.0 / D), (8, T))
            sq = None
            for r in range(0, D, 64):
                x = xg[ca + z, r:r + 64, :] - rows8(mean, 64)
                a = vsum(x * x)
                sq = a if sq is None else sq + a
                yield 24
            var = jnp.sum(sq, axis=0, keepdims=True) * (1.0 / D)
            return mean, jnp.broadcast_to(ALPHA * lax.rsqrt(var + (2.0 * ALPHA) ** 2 * EPS), (8, T))

        def ln1(c):
            if isinstance(c, int):
                cs, gpar, ca, xg = slice(c * T, (c + 1) * T), (c // 4) % 2, c % 4, X1[c // 4]
            else:
                cs, gpar, ca, xg = pl.ds(pl.multiple_of(c * T, T), T), 0, c, X1[0]
            def g():
                sm = gl = None
                for r in range(0, RG, 4):
                    x = q_v[r:r + 4, :, cs].astype(f32).reshape(64, T) * (2.0 * ALPHA)
                    xg[ca, 16 * r:16 * r + 64, :] = x
                    a, b = vsum(x), vsum(x * coef[5, r:r + 4].reshape(64, T))
                    sm = a if sm is None else sm + a
                    gl = b if gl is None else gl + b
                    yield 40
                gate = jax.nn.sigmoid(jnp.sum(gl, axis=0, keepdims=True) * (0.5 / ALPHA))
                g_v[0, :, cs] = jnp.broadcast_to(gate, (8, T))
                g_v[1, :, cs] = jnp.broadcast_to((1.0 - gate) * (0.5 / ALPHA), (8, T))
                mean, rs = yield from centred_scale(xg, ca, sm, zero[0])
                for r in range(0, D, 64):
                    XN[gpar][ca, r:r + 64, :] = ((xg[ca + zero[1], r:r + 64, :] - rows8(mean, 64)) * rows8(rs, 64)).astype(bf16)
                    yield 20
            return 9 * 84, g()

        def lhs_w(wt, rows):
            r2 = slice(rows.start // 2, rows.stop // 2)
            return jnp.concatenate([packed(wt, (kt, r2)) for kt in range(4)] + [packed(wt, (4, r2))[:, :D - 4 * T]], axis=1)

        def mix1(c):
            def g():
                for qi, sh in enumerate((1, -1, 2, -2)):
                    rows = slice(qi * DQ, (qi + 1) * DQ)
                    h = jnp.dot(lhs_w(w1t, rows), packed(XN[(c // 4) % 2], (c % 4 + zero[2 + qi],)), preferred_element_type=f32)
                    HR[c + 1, rows, :] = _gelu(pltpu.roll(h, sh % T, 1)).astype(bf16)
                    yield 5 * DQ / 3
            return 5 * D / 3, g()

        def mix2(c):
            def g():
                hv = HR.bitcast(u32)
                def shifted(z):
                    parts = []
                    for qi, sh in enumerate((1, -1, 2, -2)):
                        r2 = slice(qi * DQ // 2, (qi + 1) * DQ // 2)
                        own, nbr = hv[c + 1 + z, r2, :], hv[(c if sh > 0 else c + 2) + z, r2, :]
                        parts.append(jnp.where(lane72 >= sh if sh > 0 else lane72 < T + sh, own, nbr))
                    return pltpu.bitcast(jnp.concatenate(parts, axis=0), bf16)
                rhs = shifted(0)
                for qi in range(4):
                    rows = slice(qi * DQ, (qi + 1) * DQ)
                    X1[c // 4][c % 4, rows, :] += jnp.dot(lhs_w(w2t, rows), rhs, preferred_element_type=f32)
                    yield 5 * DQ / 3
            return 5 * D / 3, g()

        def acc_zero(g_):
            for i in BLANK:
                acc[g_, i, 0:DQ] = jnp.zeros((DQ, T), f32)
            yield 0

        def ln2(c):
            def g():
                sm = None
                for r in range(0, D, 96):
                    a = vsum(X1[c // 4][c % 4, r:r + 96, :])
                    sm = a if sm is None else sm + a
                    yield 12
                mean, rs = yield from centred_scale(X1[c // 4], c % 4, sm, zero[6])
                for kt in range(5):
                    n = T if kt < 4 else D - 4 * T
                    x = (X1[c // 4][c % 4 + zero[7], kt * T:kt * T + n, :] - rows8(mean, n)) * rows8(rs, n)
                    if n < T:
                        XE[c // 4, c % 4] = jnp.concatenate([x, jnp.zeros((T - n, T), f32)], axis=0).T.astype(bf16)
                    else:
                        XT[c % 8, kt] = x.T
                    yield 40
            return 72 + 216 + 200, g()

        def xcomb16(g_, r):
            rs = slice(r, r + 16) if isinstance(r, int) else pl.ds(pl.multiple_of(r, 16), 16)
            blk = [[XT[(4 * g_ + a) % 8, k, rs, :] for k in range(4)] for a in range(4)]
            def store(i, val):
                XS[g_, i, r // 16] = val
            yield from combos16(A_TAB, blk, store)

        def xcomb(g_):
            def g():
                for r in range(0, T, 16):
                    yield from xcomb16(g_, r)
            return 8 * 7 * wc, g()

        def acc_init(g_):
            def g():
                for r in range(0, DQ, 24):
                    blk = [[X1[g_][a, dq * DQ + r:dq * DQ + r + 24, :] for a in range(4)] for dq in range(4)]
                    for i in range(7):
                        if E_TAB[i] is not None:
                            inner = [_comb(E_TAB[i], [blk[_blk(o, p)[0]][_blk(o, p)[1]] for o in range(4)]) for p in range(4)]
                            for j in range(7):
                                if E_TAB[j] is not None:
                                    acc[g_, 7 * i + j, r:r + 24, :] = _comb(E_TAB[j], inner)
                            yield 24
            return 6 * 4 * 24, g()

        def wcomb3(pieces):
            def g():
                for t, slot, kt, r in pieces:
                    blk = [[w3_v[8 * k + r, :, pl.ds(pl.multiple_of(t * FC + KT * T * f + T * kt, T), T)].astype(f32)
                            for f in range(4)] for k in range(4)]
                    yield wl
                    def store(i, val):
                        W3C[slot, i, kt, r] = val
                    yield from combos16(B_TAB, blk, store)
            return len(pieces) * (wl + 7 * wc), g()

        def wrest(t, slot, kt):
            def g():
                for r in range(4):
                    w = [w3_v[32 + r, :, pl.ds(pl.multiple_of(t * FC + KT * T * f + T * kt, T), T)].astype(f32) for f in range(4)]
                    for c1, row in enumerate(((w[0], w[1]), (w[2], w[3]), (w[0] + w[2], w[1] + w[3]))):
                        for c2, val in enumerate((row[0], row[1], row[0] + row[1])):
                            WR[slot, kt, 3 * c1 + c2, r] = val.astype(bf16)
                    yield 30
            return 120, g()

        def wcomb4(pieces):
            def g():
                for t, slot, kt, r in pieces:
                    blk = [[w4_v[9 * dq + r, :, pl.ds(pl.multiple_of(t * FC + KT * T * f + T * kt, T), T)].astype(f32)
                            for f in range(4)] for dq in range(4)]
                    yield wl
                    def store(i, val):
                        W4C[slot, i, kt, r] = val
                    yield from combos16(A_TAB, blk, store)
            return len(pieces) * (wl + 7 * wc), g()

        def mm1(par, t, g_, kts=(0, 1, 2)):
            def g():
                for kt in kts:
                    for i in range(49):
                        m = jnp.dot(packed(XS, (g_, i, slice(0, 8))), packed(W3C, (t % 2, i, kt, slice(0, 8))),
                                    preferred_element_type=f32)
                        r1, r2 = R_TAB[i // 7], R_TAB[i % 7]
                        rest = r1 is not None and r2 is not None
                        if rest:
                            m = m + jnp.dot(packed(XE, (g_, 2 * r1[0] + r2[0]))[:, :64], packed(WR, (t % 2, kt, 3 * r1[1] + r2[1])),
                                            preferred_element_type=f32)
                        P[par][i, kt, 0:T] = m
                        yield T * (1 + rest) / KT
            return 65 * T * len(kts) / KT, g()

        def gelu8(par, kt, r):
            h = yield from recombine8(lambda i: P[par][i, kt, r:r + 8, :])
            for a in range(4):
                for f in range(4):
                    h[a][f] = _gelu(h[a][f])
                yield wg
            return h

        def act(par, dst):
            def g():
                for kt in range(KT):
                    for r in range(0, T, 16):
                        h0 = yield from gelu8(par, kt, r)
                        h1 = yield from gelu8(par, kt, r + 8)
                        blk = [[jnp.concatenate([h0[a][f], h1[a][f]], axis=0) for a in range(4)] for f in range(4)]
                        def store(i, val):
                            dst[i, kt, r:r + 16, :] = val
                        yield from combos16(B_TAB, blk, store)
            return 24 * (2 * (7 * wr + 4 * wg) + 7 * wc), g()

        def mm2(slot, g_, src, lo=0, hi=49, kts=(0, 1, 2)):
            def g():
                for i in range(lo, hi):
                    lhs = jnp.concatenate([packed(W4C, (slot, i, kt, slice(0, 9))) for kt in kts], axis=1)
                    rhs = jnp.concatenate([packed(src, (i, kt, slice(0, T // 2))) for kt in kts], axis=1)
                    acc[g_, i, 0:DQ] += lax.dot_general(lhs, rhs, NT_DIMS, preferred_element_type=f32)
                    yield DQ * len(kts) / 3
            return (hi - lo) * DQ * len(kts) / 3, g()


        def conv_kv(c, slot_=None):
            def g():
                for l in range(CG):
                    rg = c * CG + l
                    cf = [coef[j, rg] for j in range(4)]
                    prev = None
                    for tt in range(NTILE):
                        cs = slice(tt * T, (tt + 1) * T)
                        kk = k_v[rg, :, cs].astype(f32)
                        rolled = [pltpu.roll(kk * cf[j], j, 1) for j in (1, 2, 3)]
                        ks = kk * cf[0]
                        for j in (1, 2, 3):
                            ks = ks + jnp.where(lane16 >= j, rolled[j - 1], 0.0 if prev is None else prev[j - 1])
                        prev = rolled
                        KV[c % 2 if slot_ is None else slot_, l, tt * 16:(tt + 1) * 16, :] = (ks * v_v[rg, :, cs].astype(f32)).astype(bf16)
                        yield 27
            return CG * NTILE * 27, g()

        def conv_fwd(c, par):
            def g():
                def fm(z):
                    return jnp.concatenate([packed(fwd_v, (z,)), packed(fwd_v, (z + 1,))], axis=1)
                for l in range(CG):
                    rg = c * CG + l
                    z = jnp.dot(packed(KV, (par, l)), fm(zero[2 * l]), preferred_element_type=f32)
                    zr, zi = z[:, :T], z[:, T:]
                    Z[par * CG + l, 0, 0:16 * NTILE] = zr
                    Z[par * CG + l, 1, 0:16 * NTILE] = zi
                    if gauss:
                        Z[par * CG + l, 4, 0:16 * NTILE] = zr + zi
                    yield 512 / 3
                    lhs = jnp.concatenate([f_v[rg, :, m * T:(m + 1) * T] for m in range(NTILE)], axis=0)
                    z = jnp.dot(lhs, fm(zero[2 * l + 1]), preferred_element_type=f32)
                    for m in range(NTILE):
                        kr, ki = z[16 * m:16 * m + 16, :T], z[16 * m:16 * m + 16, T:]
                        if m == 0:
                            kr = kr + coef[4, rg]
                        else:
                            sigma = sign[...]
                            kr = kr - sigma * z[16 * m - 16:16 * m, T:]
                            ki = ki + sigma * z[16 * m - 16:16 * m, :T]
                        if gauss:
                            Z[par * CG + l, 2, 16 * m:16 * m + 16] = kr
                            Z[par * CG + l, 3, 16 * m:16 * m + 16] = ki - kr
                            Z[par * CG + l, 5, 16 * m:16 * m + 16] = ki + kr
                        else:
                            Z[par * CG + l, 2, 16 * m:16 * m + 16] = kr
                            Z[par * CG + l, 3, 16 * m:16 * m + 16] = ki
                    yield 512 / 3
            return CG * 1024 / 3, g()

        def conv_pw_block(par, l, b):
            i0 = b * nb
            w = 12 if gauss else 16
            def g():
                lz = par * CG + l + zero[b % 8]
                def z(kind, j):
                    return Z[lz, kind, 16 * j:16 * j + 16]
                yr = {}
                for j in range(i0 + nb):
                    ur, ui = z(0, j), z(1, j)
                    for i in range(max(i0, j), i0 + nb):
                        if gauss:
                            p = (z(2, i - j) * z(4, j), ur * z(3, i - j), ui * z(5, i - j))
                        else:
                            kr, ki = z(2, i - j), z(3, i - j)
                            p = (ur * kr - ui * ki, ur * ki + ui * kr)
                        yr[i] = p if i not in yr else tuple(x + y for x, y in zip(yr[i], p))
                    yield w * (i0 + nb - max(i0, j))
                for i in range(i0, i0 + nb):
                    re, im = (yr[i][0] - yr[i][2], yr[i][0] + yr[i][1]) if gauss else yr[i]
                    Y[l, 0, 16 * i:16 * i + 16, :] = re.astype(bf16)
                    Y[l, 1, 16 * i:16 * i + 16, :] = im.astype(bf16)
            return w * sum(i + 1 for i in range(i0, i0 + nb)), g()

        def conv_pw(par):
            return _chain(*[conv_pw_block(par, l, b) for l in range(CG) for b in range(NTILE // nb)])

        def conv_inv(c):
            def g():
                for l in range(CG):
                    rg = c * CG + l
                    lhs = jnp.concatenate([packed(Y, (l, 0, slice(0, 8 * NTILE))), packed(Y, (l, 1, slice(0, 8 * NTILE)))], axis=1)
                    y = jnp.dot(lhs, packed(inv_v, (zero[l],)), preferred_element_type=f32)
                    for i in range(NTILE):
                        cs = slice(i * T, (i + 1) * T)
                        gate = g_v[0, :, cs]
                        ga[rg, :, cs] = y[16 * i:16 * i + 16] * (q_v[rg, :, cs].astype(f32) * jnp.concatenate([gate, gate], axis=0))
                    yield 512 / 3
            return CG * 512 / 3, g()

        def final16(g_, r16):
            w = [g_v[1, :, (4 * g_ + a) * T:(4 * g_ + a + 1) * T] for a in range(4)]
            for half in (0, 8):
                r = r16 * 16 + half
                rs = slice(r, r + 8) if isinstance(r, int) else pl.ds(pl.multiple_of(r, 8), 8)
                h = yield from recombine8(lambda i: acc[g_, i, rs, :])
                for dq in range(4):
                    for a in range(4):
                        idx = (9 * dq + r16, slice(half, half + 8), slice((4 * g_ + a) * T, (4 * g_ + a + 1) * T))
                        o_v[idx] = (ga[idx] + w[a] * h[dq][a]).astype(bf16)
                    yield 12

        def final(groups):
            def g():
                for r16 in range(9):
                    for g_ in groups:
                        yield from final16(g_, r16)
            return len(groups) * 18 * (7 * wr + 48), g()

        def out_copy(g_):
            sl = pl.ds(g_ * 4 * T, 4 * T)
            return pltpu.make_async_copy(o_v.at[:, :, sl], out_hbm.at[:, :, sl], osems.at[g_])

        def action(fn, *a):
            def g():
                fn(*a)
                yield 0
            return 0, g()

        def block(fn):
            @pl.when(zs[15] == 0)
            def _():
                load_zeros()
                fn()

        def tiles(fn, g_):
            return _chain(*[fn(4 * g_ + a) for a in range(4)])

        def w3p(t, lo, hi):
            return wcomb3([(t, t % 2, pc // 8, pc % 8) for pc in range(lo, hi)])

        def w4p(t, lo, hi):
            return wcomb4([(t, t % 2, pc // 9, pc % 9) for pc in range(lo, hi)])

        nslot = [0]

        def slot(mxu, vpu, sk=sk1, fill=None):
            nslot[0] += 1
            if nslot[0] <= upto and (only is None or nslot[0] in only):
              with scope('slot%02d' % nslot[0]):
                block(lambda: _interleave(_chain(*mxu()), _chain(*vpu()) + (0.0, sk), *([_chain(*fill())] if fill else [])))

        def loop(n, piece):
            def body(i, carry):
                _run((0, piece(i)))
                return carry
            lax.fori_loop(0, n, body, 0)

        load_zeros()
        wait('gw', 'sk', 'd')
        _run(coefs([5, 0, 1, 2, 3, 4]))
        loop(1, acc_zero)
        wait('q0')
        loop(4, lambda c: ln1(c)[1])
        loop(1, lambda i: acc_zero(i + 1))
        wait('w1')
        _run(transpose_w(w1_v, w1t))
        loop(1, lambda i: acc_zero(i + 2))
        wait('q1')
        slot(lambda: [tiles(mix1, 0)], lambda: [tiles(ln1, 1)])
        wait('q2', 'w2')
        slot(lambda: [tiles(mix1, 1)], lambda: [transpose_w(w2_v, w2t), tiles(ln1, 2)])
        loop(1, lambda i: acc_zero(i + 3))
        wait('q3', *w3_a)
        slot(lambda: [tiles(mix1, 2), tiles(mix2, 0)], lambda: [tiles(ln1, 3), w3p(0, 0, 8), wrest(0, 0, 0)])
        wait('k0', 'v0', *w3_b)
        c4 = [(0, 3, 9), (0, 6, 15), (0, 3, 12), (0, 5, 12)][pv]
        slot(lambda: [tiles(mix1, 3), tiles(mix2, 1)], lambda: [conv_kv(0), conv_kv(1), tiles(ln2, 0), acc_init(0), w3p(0, 8, 24), wrest(0, 0, 1), wrest(0, 0, 2)])
        wait('w4_0')
        slot(lambda: [tiles(mix2, 2)], lambda: [tiles(ln2, 1), acc_init(1), xcomb(0), w4p(0, c4[0], c4[1])])
        wait('f0', 'fwd', 'inv', 'w3_1')
        slot(lambda: [conv_fwd(0, 0), tiles(mix2, 3), conv_fwd(1, 1)],
             lambda: [tiles(ln2, 2), acc_init(2), xcomb(1), w4p(0, c4[1], c4[2]), w3p(1, 0, 6)])
        slot(lambda: [mm1(0, 0, 0)], lambda: [tiles(ln2, 3), acc_init(3), xcomb(2), conv_kv(2), w4p(0, c4[2], 21), conv_pw(0)])
        loop(8, lambda i: xcomb16(3, i * 16))
        wait('f', 'k', 'v', 'w4_1')

        def stage_a(s, par):
            tn, j = (s + 2) // NTG, (s + 2) % NTG
            p4 = []
            for n in range(7):
                pc = jnp.minimum(j * 7 + n, 26)
                p4.append((jnp.minimum(tn, NFC - 1), tn % 2, pc // 9, pc % 9))
            ci, cf, m1 = conv_inv(s - 1), conv_fwd(jnp.minimum(s + 1, NU - 1), 1 - par), mm1(par, s // NTG, s % NTG)
            _interleave(_chain(*[(ci, cf, m1), (cf, ci, m1), (cf, m1, ci), (m1, cf, ci), (ci, m1, cf)][ca]),
                        _chain(act(1 - par, B), wcomb4(p4)) + (0.0, ska))

        def stage_b(s):
            tn, j = s // NTG + 1, s % NTG
            p3 = []
            for n in range(6):
                pc = j * 6 + n
                p3.append((jnp.minimum(tn, NFC - 1), tn % 2, pc // 8, pc % 8))
            _interleave(mm2(((s - 1) // NTG) % 2, (s - 1) % NTG, B),
                        _chain(conv_kv(jnp.minimum(s + 2, NU - 1)), wcomb3(p3), wrest(jnp.minimum(tn, NFC - 1), tn % 2, jnp.maximum(j - 1, 0)),
                               conv_pw(s % 2)) + (0.0, skb))

        def stage(s, carry):
            pl.when(s == NTG)(lambda: wait('w3_2', 'w4_2'))
            for par in range(2):
                load_zeros()
                with scope('A%d' % par):
                    pl.when(s % 2 == par)(lambda: stage_a(s, par))
            with scope('B'):
                pl.when(s < NU - 1)(lambda: stage_b(s))
            return carry

        if upto > 7 and (only is None or 0 in only):
            lax.fori_loop(1, NU, stage, 0)

        last, sl, gl = (NU - 1) % 2, (NFC - 1) % 2, NTG - 1
        slot(lambda: [mm2(sl + zero[0], gl - 1 + zero[0], B)], lambda: [act(last, B2)], 0.95)
        slot(lambda: [mm2(sl + zero[0], gl + zero[0], B2, 0, esplit)], lambda: [conv_pw(last)])
        cuts = [esplit + (49 - esplit - e2) * n // 3 for n in range(3)] + [49]
        for g_ in range(3):
            slot(lambda: ([conv_inv(NU - 1)] if g_ == 0 else []) + [mm2(sl + zero[0], gl, B2, cuts[g_], cuts[g_ + 1])],
                 lambda: [final((g_,))], 0.97)
            out_copy(g_).start()

        def band(n, dq):
            rows, cols = pl.ds(9 * dq + 3 * n, 3), pl.ds(gl * 4 * T, 4 * T)
            return pltpu.make_async_copy(o_v.at[rows, :, cols], out_hbm.at[rows, :, cols], bsems.at[n, dq])

        def tail(n, carry):
            for r in range(3):
                _run((0, final16(gl, 3 * n + r)))
            for dq in range(4):
                band(n, dq).start()
            return carry

        lax.fori_loop(0, 3, tail, 0)
        with scope('out_wait'):
            for g_ in range(3):
                out_copy(g_).wait()
            for n in range(3):
                for dq in range(4):
                    band(n, dq).wait()

    def fn(A_q, A_k, A_v, A_shift_k, A_ssm_k, A_ssm_D, B_x, B_w1, B_w2, B_w3, B_w4, gate_w):
        del B_x
        fwd, inv = _dft_mats()
        hbm = pl.BlockSpec(memory_space=pl.ANY)
        V = pltpu.VMEM
        out = pl.pallas_call(
            kernel,
            out_shape=jax.ShapeDtypeStruct((RG, 16, S), bf16),
            in_specs=[hbm] * 13,
            out_specs=hbm,
            scratch_shapes=[
                V((RG, 16, S), bf16), V((RG, 16, S), bf16), V((RG, 16, S), bf16), V((RG, 16, S), bf16),
                V((D, D), bf16), V((D, D), bf16), V((RG, 16, F), bf16), V((RG, 16, F), bf16),
                V((4, D), bf16), V((D,), bf16), V((D,), bf16), V((2, T, T), bf16), V((1, 2 * T, T), bf16),
                V((5, D, T), bf16), V((5, D, T), bf16),
                V((6, RG, 16, T), f32), V((16, T), f32),
                V((2, 8, S), f32),
                V((4, D, T), bf16), V((4, D, T), bf16),
                V((NTILE + 2, D, T), bf16),
                V((4, D, T), f32), V((4, D, T), f32), V((4, D, T), f32), V((4, D, T), f32),
                V((8, 4, T, T), f32),
                V((NTG, 49, 8 + px, 16, T), bf16), V((NTG, 4, T, T), bf16),
                V((2, KT, 9, 4, 16, T), bf16),
                V((2, 49, KT, 8 + pw, 16, T), bf16),
                V((2, 49, KT, 9 + p4, 16, T), bf16),
                V((49, KT, T + pp, T), f32), V((49, KT, T + pp, T), f32),
                V((49, KT, T + pb, T), bf16), V((49, KT, T + pb, T), bf16),
                V((NTG, 49, DQ + pa, T), f32),
                V((2, CG, 16 * NTILE, T), bf16),
                V((2 * CG, 6 if gauss else 4, NTILE * 16 + pz, T), f32),
                V((CG, 2, 16 * NTILE + py, T), bf16),
                V((RG, 16, S), f32),
                V((RG, 16, S), bf16),
                pltpu.SMEM((16,), jnp.int32),
                pltpu.SemaphoreType.DMA((32,)),
                pltpu.SemaphoreType.DMA((NTG - 1,)),
                pltpu.SemaphoreType.DMA((3, 4)),
            ],
            compiler_params=pltpu.CompilerParams(vmem_limit_bytes=126 * 1024 * 1024),
        )(A_q[0].T.reshape(RG, 16, S), A_k[0].T.reshape(RG, 16, S), A_v[0].T.reshape(RG, 16, S), A_shift_k.T,
          A_ssm_k.reshape(RG, 16, S), A_ssm_D, B_w1, B_w2, B_w3.reshape(RG, 16, F), B_w4.T.reshape(RG, 16, F), gate_w,
          fwd, inv)
        return out.reshape(D, S).T[None]
    return fn


pallas_gated_mix__ssm_conv_h3__mixer_s_mlp__prompt_kernel = jax.jit(make())
```

```python
import numpy as np
import ml_dtypes
import jax
import jax.numpy as jnp
from jax import lax
import jax.experimental.pallas as pl
import jax.experimental.pallas.tpu as pltpu

S, D, F = 2048, 576, 4608
T = 128
NTILE = S // T
RG = D // 16
KT = 3
FC = 4 * KT * T
NFC = F // FC
NTG = NTILE // 4
NU = NFC * NTG
CG = RG // NU
DQ = D // 4
DR = D - 4 * T
EPS = 1e-5
GELU_C0 = float(np.sqrt(2.0 / np.pi))
ALPHA = float((0.044715 * GELU_C0) ** (1.0 / 3.0))
f32, bf16, u32 = jnp.float32, jnp.bfloat16, jnp.uint32
SHIFTS = (1, -1, 2, -2)

A_TAB = (((1, 0), (1, 3)), ((1, 2), (1, 3)), ((1, 0),), ((1, 3),), ((1, 0), (1, 1)), ((1, 2), (-1, 0)), ((1, 1), (-1, 3)))
B_TAB = (((1, 0), (1, 3)), ((1, 0),), ((1, 1), (-1, 3)), ((1, 2), (-1, 0)), ((1, 3),), ((1, 0), (1, 1)), ((1, 2), (1, 3)))
C_TAB = (((1, 0), (1, 3)), ((1, 2), (-1, 3)), ((1, 1), (1, 3)), ((1, 0), (1, 2)), ((-1, 0), (1, 1)), ((1, 3),), ((1, 0),))
E_TAB = (None, ((1, 2),), ((1, 1),), None, None, ((1, 3), (-1, 1), (1, 2)), ((1, 0),))
BLANK = [7 * i + j for i in range(7) for j in range(7) if E_TAB[i] is None or E_TAB[j] is None]
R_TAB = (None, (1, 0), None, None, (0, 1), (1, 2), (0, 2))

PLAN = {
    "s1": (0.00, 0.98, 13, 30, 35, 32), "s2": (0.01, 0.98, 12, 30, 35, 32), "s3": (0.00, 0.99, 13, 30, 35, 32),
    "s4": (0.01, 0.86, 9, 40, 37, 32), "s5": (0.00, 0.97, 10, 24, 39, 34), "s6": (0.00, 0.86, 19, 38, 41, 43),
    "s7": (0.08, 1.03, 14, 29, 50, 16), "a": (0.04, 0.93, 10, 29, 53, 23), "b": (0.03, 0.99, 13, 30, 35, 27),
    "e1": (0.02, 0.99, 10, 56, 50, 32), "e2": (0.02, 1.01, 13, 30, 35, 32), "f0": (0.00, 1.05, 13, 22, 35, 32),
    "f1": (0.01, 0.96, 13, 41, 24, 32), "f2": (0.01, 0.96, 13, 30, 30, 32),
}
LAST_CUTS = (21, 26, 34, 42)


def _dft_matrices():
    n = np.arange(T, dtype=np.float64)[:, None]
    f = np.arange(T, dtype=np.float64)[None, :]
    theta = 2.0 * np.pi * (f + 0.5) * n / (2 * T)
    fwd = np.stack([np.cos(theta), -np.sin(theta)])
    inv = np.concatenate([fwd[0].T, fwd[1].T])[None] / T
    return fwd.astype(ml_dtypes.bfloat16), inv.astype(ml_dtypes.bfloat16)


def _comb(tab, quad):
    (_, first), *rest = tab
    v = quad[first]
    for sign, o in rest:
        v = v + quad[o] if sign > 0 else v - quad[o]
    return v


def _blk(o, p):
    return 2 * (o // 2) + p // 2, 2 * (o % 2) + p % 2


def _gelu(h):
    return h * (1.0 + jnp.tanh(h * (GELU_C0 / ALPHA + h * h)))


def _chain(*streams):
    def g():
        for s in streams:
            yield from s[1]
    return sum(s[0] for s in streams), g()


def _run(*streams):
    for s in streams:
        for _ in s[1]:
            pass


def _interleave(first, second, lo, hi):
    live = [[0.0, float(first[0]) or 1.0, first[1], 0.0, 1.0], [0.0, float(second[0]) or 1.0, second[1], lo, hi]]
    while live:
        live.sort(key=lambda x: x[3] + (x[4] - x[3]) * x[0] / x[1])
        try:
            live[0][0] += next(live[0][2])
        except StopIteration:
            live.pop(0)


def _packed(ref, idx):
    v = ref.bitcast(u32)[idx]
    if v.ndim == 3:
        v = v.reshape(v.shape[0] * v.shape[1], v.shape[2])
    return pltpu.bitcast(v, bf16)


def _vsum(x):
    parts = [x[r:r + 8] for r in range(0, x.shape[0], 8)]
    while len(parts) > 1:
        parts = [parts[i] + parts[i + 1] for i in range(0, len(parts) - 1, 2)] + ([parts[-1]] if len(parts) % 2 else [])
    return parts[0]


def _rows(stat, n):
    return jnp.concatenate([stat] * (n // 8), axis=0)


def _kernel(q_hbm, k_hbm, v_hbm, sk_hbm, f_hbm, d_hbm, w1_hbm, w2_hbm, w3_hbm, w4_hbm, gw_hbm, fwd_hbm, inv_hbm,
            out_hbm,
            q_v, k_v, v_v, f_v, w1_v, w2_v, w3_v, w4_v, sk_v, d_v, gw_v, fwd_v, inv_v,
            w1t, w2t, coef, sign, gate, xn0, xn1, HR, x1a, x1b, x1c, x1d, XT, XS, XE, WR, W3C, W4C, p0, p1, B, B2, acc,
            KV, Z, Y, ga, o_v, zs, in_sems, out_sems, band_sems):
    XN, X1, P = (xn0, xn1), (x1a, x1b, x1c, x1d), (p0, p1)
    every = slice(None)
    weight = {}
    zero = []

    pairs = dict(gw=(gw_hbm, gw_v), sk=(sk_hbm, sk_v), d=(d_hbm, d_v), w1=(w1_hbm, w1_v), w2=(w2_hbm, w2_v),
                 fwd=(fwd_hbm, fwd_v), inv=(inv_hbm, inv_v))

    def part(name, src, dst, idx):
        pairs[name] = (src.at[idx], dst.at[idx])

    for g_ in range(NTG):
        part("q%d" % g_, q_hbm, q_v, (every, every, pl.ds(g_ * 4 * T, 4 * T)))
    for name, src, dst, first in (("k", k_hbm, k_v, 4 * CG), ("v", v_hbm, v_v, 4 * CG), ("f", f_hbm, f_v, 3 * CG)):
        part(name + "0", src, dst, pl.ds(0, first))
        part(name, src, dst, pl.ds(first, RG - first))
    for fq in range(4):
        part("w3_a%d" % fq, w3_hbm, w3_v, (every, every, pl.ds(fq * KT * T, 2 * T)))
        part("w3_b%d" % fq, w3_hbm, w3_v, (every, every, pl.ds(fq * KT * T + 2 * T, T)))
    for t in range(NFC):
        if t:
            part("w3_%d" % t, w3_hbm, w3_v, (every, every, pl.ds(t * FC, FC)))
        part("w4_%d" % t, w4_hbm, w4_v, (every, every, pl.ds(t * FC, FC)))
    w3_a, w3_b = ["w3_a%d" % fq for fq in range(4)], ["w3_b%d" % fq for fq in range(4)]
    early = ["gw", "sk", "d", "w1", "q0", "q1", "w2", "q2", "q3"] + w3_a + ["k0", "v0"] + w3_b \
        + ["w4_0", "f0", "fwd", "inv", "w3_1"]
    later = ["w4_1", "f", "k", "v", "w3_2", "w4_2"]
    copies = {n: pltpu.make_async_copy(pairs[n][0], pairs[n][1], in_sems.at[i]) for i, n in enumerate(early + later)}

    def start(*names):
        for n in names:
            copies[n].start()

    def wait(*names):
        for n in names:
            copies[n].wait()

    start(*early)
    for i in range(16):
        zs[i] = 0
    HR[0] = jnp.zeros((D, T), bf16)
    HR[NTILE + 1] = jnp.zeros((D, T), bf16)
    lane16 = lax.broadcasted_iota(jnp.int32, (16, T), 1)
    lane72 = lax.broadcasted_iota(jnp.int32, (DQ // 2, T), 1)
    sign[...] = (1 - 2 * (lane16 & 1)).astype(f32)

    def load_zeros():
        zero[:] = [zs[i] for i in range(16)]

    def combos16(tab, blk, store):
        for i in range(7):
            inner = [_comb(tab[i], [blk[_blk(o, p)[0]][_blk(o, p)[1]] for o in range(4)]) for p in range(4)]
            for j in range(7):
                store(7 * i + j, _comb(tab[j], inner).astype(bf16))
            yield weight["comb"]

    def recombine8(load):
        h = [[None] * 4 for _ in range(4)]
        for i in range(7):
            m = [load(7 * i + j) for j in range(7)]
            quad = [m[0] + m[3] - m[4] + m[6], m[2] + m[4], m[1] + m[3], m[0] - m[1] + m[2] + m[5]]
            for s, o in C_TAB[i]:
                for p in range(4):
                    a, b = _blk(o, p)
                    if h[a][b] is None:
                        h[a][b] = quad[p] if s > 0 else -quad[p]
                    else:
                        h[a][b] = h[a][b] + quad[p] if s > 0 else h[a][b] - quad[p]
            yield weight["recombine"]
        return h

    def transpose_w(src, dst):
        def g():
            for kt in range(5):
                n = T if kt < 4 else DR
                w = src[kt * T:kt * T + n, :].astype(f32)
                if n < T:
                    w = jnp.concatenate([w, jnp.zeros((T - n, D), f32)], axis=0)
                dst[kt] = w.T.astype(bf16)
                yield 100
        return 500, g()

    def set_coefs():
        for i in (5, 0, 1, 2, 3, 4):
            if i < 4:
                row = sk_v[...].astype(f32)[i:i + 1]
            else:
                row = (d_v if i == 4 else gw_v)[...].astype(f32).reshape(1, D)
            coef[i] = jnp.broadcast_to(row, (T, D)).T.reshape(RG, 16, T)

    def centred_scale(xg, a, total, z):
        mean = jnp.broadcast_to(jnp.sum(total, axis=0, keepdims=True) * (1.0 / D), (8, T))
        sq = None
        for r in range(0, D, 64):
            x = xg[a + z, r:r + 64, :] - _rows(mean, 64)
            part_sq = _vsum(x * x)
            sq = part_sq if sq is None else sq + part_sq
            yield 24
        var = jnp.sum(sq, axis=0, keepdims=True) * (1.0 / D)
        return mean, jnp.broadcast_to(ALPHA * lax.rsqrt(var + (2.0 * ALPHA) ** 2 * EPS), (8, T))

    def ln1(c):
        if isinstance(c, int):
            cols, xn, xg, a = slice(c * T, (c + 1) * T), XN[(c // 4) % 2], X1[c // 4], c % 4
        else:
            cols, xn, xg, a = pl.ds(pl.multiple_of(c * T, T), T), XN[0], X1[0], c

        def g():
            total = logit = None
            for r in range(0, RG, 4):
                x = q_v[r:r + 4, :, cols].astype(f32).reshape(64, T) * (2.0 * ALPHA)
                xg[a, 16 * r:16 * r + 64, :] = x
                s, l = _vsum(x), _vsum(x * coef[5, r:r + 4].reshape(64, T))
                total = s if total is None else total + s
                logit = l if logit is None else logit + l
                yield 40
            g_val = jax.nn.sigmoid(jnp.sum(logit, axis=0, keepdims=True) * (0.5 / ALPHA))
            gate[0, :, cols] = jnp.broadcast_to(g_val, (8, T))
            gate[1, :, cols] = jnp.broadcast_to((1.0 - g_val) * (0.5 / ALPHA), (8, T))
            mean, scale = yield from centred_scale(xg, a, total, zero[0])
            for r in range(0, D, 64):
                xn[a, r:r + 64, :] = ((xg[a + zero[1], r:r + 64, :] - _rows(mean, 64)) * _rows(scale, 64)).astype(bf16)
                yield 20
        return 9 * 84, g()

    def lhs_w(wt, rows):
        r2 = slice(rows.start // 2, rows.stop // 2)
        return jnp.concatenate([_packed(wt, (kt, r2)) for kt in range(4)] + [_packed(wt, (4, r2))[:, :DR]], axis=1)

    def mix1(c):
        def g():
            for qi, sh in enumerate(SHIFTS):
                rows = slice(qi * DQ, (qi + 1) * DQ)
                h = jnp.dot(lhs_w(w1t, rows), _packed(XN[(c // 4) % 2], (c % 4 + zero[2 + qi],)), preferred_element_type=f32)
                HR[c + 1, rows, :] = _gelu(pltpu.roll(h, sh % T, 1)).astype(bf16)
                yield 5 * DQ / 3
        return 5 * D / 3, g()

    def mix2(c):
        def g():
            hv = HR.bitcast(u32)
            parts = []
            for qi, sh in enumerate(SHIFTS):
                r2 = slice(qi * DQ // 2, (qi + 1) * DQ // 2)
                own, neighbour = hv[c + 1, r2, :], hv[c if sh > 0 else c + 2, r2, :]
                parts.append(jnp.where(lane72 >= sh if sh > 0 else lane72 < T + sh, own, neighbour))
            rhs = pltpu.bitcast(jnp.concatenate(parts, axis=0), bf16)
            for qi in range(4):
                rows = slice(qi * DQ, (qi + 1) * DQ)
                X1[c // 4][c % 4, rows, :] += jnp.dot(lhs_w(w2t, rows), rhs, preferred_element_type=f32)
                yield 5 * DQ / 3
        return 5 * D / 3, g()

    def ln2(c):
        xg, a = X1[c // 4], c % 4

        def g():
            total = None
            for r in range(0, D, 96):
                s = _vsum(xg[a, r:r + 96, :])
                total = s if total is None else total + s
                yield 12
            mean, scale = yield from centred_scale(xg, a, total, zero[6])
            for kt in range(5):
                n = T if kt < 4 else DR
                x = (xg[a + zero[7], kt * T:kt * T + n, :] - _rows(mean, n)) * _rows(scale, n)
                if n < T:
                    XE[c // 4, a] = jnp.concatenate([x, jnp.zeros((T - n, T), f32)], axis=0).T.astype(bf16)
                else:
                    XT[c % 8, kt] = x.T
                yield 40
        return 72 + 216 + 200, g()

    def xcomb(g_):
        def g():
            for r in range(0, T, 16):
                blk = [[XT[(4 * g_ + a) % 8, kt, r:r + 16, :] for kt in range(4)] for a in range(4)]

                def store(i, val):
                    XS[g_, i, r // 16] = val
                yield from combos16(A_TAB, blk, store)
        return 8 * 7 * weight["comb"], g()

    def acc_zero(g_):
        for i in BLANK:
            acc[g_, i, 0:DQ] = jnp.zeros((DQ, T), f32)
        yield 0

    def acc_init(g_):
        def g():
            for r in range(0, DQ, 24):
                blk = [[X1[g_][a, dq * DQ + r:dq * DQ + r + 24, :] for a in range(4)] for dq in range(4)]
                for i in range(7):
                    if E_TAB[i] is not None:
                        inner = [_comb(E_TAB[i], [blk[_blk(o, p)[0]][_blk(o, p)[1]] for o in range(4)]) for p in range(4)]
                        for j in range(7):
                            if E_TAB[j] is not None:
                                acc[g_, 7 * i + j, r:r + 24, :] = _comb(E_TAB[j], inner)
                        yield 24
        return 6 * 4 * 24, g()

    def feature_tile(t, fq, kt):
        return pl.ds(pl.multiple_of(t * FC + KT * T * fq + T * kt, T), T)

    def wcomb3(pieces):
        def g():
            for t, slot, kt, r in pieces:
                blk = [[w3_v[8 * k + r, :, feature_tile(t, fq, kt)].astype(f32) for fq in range(4)] for k in range(4)]
                yield weight["load"]

                def store(i, val):
                    W3C[slot, i, kt, r] = val
                yield from combos16(B_TAB, blk, store)
        return len(pieces) * (weight["load"] + 7 * weight["comb"]), g()

    def wrest(t, slot, kt):
        def g():
            for r in range(4):
                w = [w3_v[32 + r, :, feature_tile(t, fq, kt)].astype(f32) for fq in range(4)]
                for c1, row in enumerate(((w[0], w[1]), (w[2], w[3]), (w[0] + w[2], w[1] + w[3]))):
                    for c2, val in enumerate((row[0], row[1], row[0] + row[1])):
                        WR[slot, kt, 3 * c1 + c2, r] = val.astype(bf16)
                yield 30
        return 120, g()

    def wcomb4(pieces):
        def g():
            for t, slot, kt, r in pieces:
                blk = [[w4_v[9 * dq + r, :, feature_tile(t, fq, kt)].astype(f32) for fq in range(4)] for dq in range(4)]
                yield weight["load"]

                def store(i, val):
                    W4C[slot, i, kt, r] = val
                yield from combos16(A_TAB, blk, store)
        return len(pieces) * (weight["load"] + 7 * weight["comb"]), g()

    def mm1(par, t, g_):
        def g():
            for kt in range(KT):
                for i in range(49):
                    m = jnp.dot(_packed(XS, (g_, i)), _packed(W3C, (t % 2, i, kt, slice(0, 8))), preferred_element_type=f32)
                    r1, r2 = R_TAB[i // 7], R_TAB[i % 7]
                    rest = r1 is not None and r2 is not None
                    if rest:
                        m = m + jnp.dot(_packed(XE, (g_, 2 * r1[0] + r2[0]))[:, :DR], _packed(WR, (t % 2, kt, 3 * r1[1] + r2[1])),
                                        preferred_element_type=f32)
                    P[par][i, kt, 0:T] = m
                    yield T * (1 + rest) / KT
        return 65 * T, g()

    def gelu8(par, kt, r):
        h = yield from recombine8(lambda i: P[par][i, kt, r:r + 8, :])
        for a in range(4):
            for fq in range(4):
                h[a][fq] = _gelu(h[a][fq])
            yield weight["gelu"]
        return h

    def act(par, dst):
        def g():
            for kt in range(KT):
                for r in range(0, T, 16):
                    h0 = yield from gelu8(par, kt, r)
                    h1 = yield from gelu8(par, kt, r + 8)
                    blk = [[jnp.concatenate([h0[a][fq], h1[a][fq]], axis=0) for a in range(4)] for fq in range(4)]

                    def store(i, val):
                        dst[i, kt, r:r + 16, :] = val
                    yield from combos16(B_TAB, blk, store)
        return 24 * (2 * (7 * weight["recombine"] + 4 * weight["gelu"]) + 7 * weight["comb"]), g()

    def mm2(slot, g_, src, lo=0, hi=49):
        def g():
            for i in range(lo, hi):
                lhs = jnp.concatenate([_packed(W4C, (slot, i, kt)) for kt in range(KT)], axis=1)
                rhs = jnp.concatenate([_packed(src, (i, kt)) for kt in range(KT)], axis=1)
                acc[g_, i, 0:DQ] += lax.dot_general(lhs, rhs, (((1,), (1,)), ((), ())), preferred_element_type=f32)
                yield DQ
        return (hi - lo) * DQ, g()

    def conv_kv(c):
        def g():
            for l in range(CG):
                rg = c * CG + l
                cf = [coef[j, rg] for j in range(4)]
                prev = None
                for tt in range(NTILE):
                    cols = slice(tt * T, (tt + 1) * T)
                    kk = k_v[rg, :, cols].astype(f32)
                    rolled = [pltpu.roll(kk * cf[j], j, 1) for j in (1, 2, 3)]
                    ks = kk * cf[0]
                    for j in (1, 2, 3):
                        ks = ks + jnp.where(lane16 >= j, rolled[j - 1], 0.0 if prev is None else prev[j - 1])
                    prev = rolled
                    KV[c % 2, l, tt * 16:(tt + 1) * 16, :] = (ks * v_v[rg, :, cols].astype(f32)).astype(bf16)
                    yield 27
        return CG * NTILE * 27, g()

    def conv_fwd(c, par):
        def g():
            def dft(z):
                return jnp.concatenate([_packed(fwd_v, (z,)), _packed(fwd_v, (z + 1,))], axis=1)
            for l in range(CG):
                rg, lz = c * CG + l, par * CG + l
                z = jnp.dot(_packed(KV, (par, l)), dft(zero[2 * l]), preferred_element_type=f32)
                Z[lz, 0, 0:16 * NTILE] = z[:, :T]
                Z[lz, 1, 0:16 * NTILE] = z[:, T:]
                yield 512 / 3
                taps = jnp.concatenate([f_v[rg, :, m * T:(m + 1) * T] for m in range(NTILE)], axis=0)
                z = jnp.dot(taps, dft(zero[2 * l + 1]), preferred_element_type=f32)
                for m in range(NTILE):
                    kr, ki = z[16 * m:16 * m + 16, :T], z[16 * m:16 * m + 16, T:]
                    if m == 0:
                        kr = kr + coef[4, rg]
                    else:
                        sigma = sign[...]
                        kr = kr - sigma * z[16 * m - 16:16 * m, T:]
                        ki = ki + sigma * z[16 * m - 16:16 * m, :T]
                    Z[lz, 2, 16 * m:16 * m + 16] = kr
                    Z[lz, 3, 16 * m:16 * m + 16] = ki
                yield 512 / 3
        return CG * 1024 / 3, g()

    def conv_bins(par):
        def g():
            for l in range(CG):
                for b, i0 in enumerate(range(0, NTILE, 2)):
                    lz = par * CG + l + zero[b % 8]
                    y = {}
                    for j in range(i0 + 2):
                        ur, ui = Z[lz, 0, 16 * j:16 * j + 16], Z[lz, 1, 16 * j:16 * j + 16]
                        for i in range(max(i0, j), i0 + 2):
                            m = 16 * (i - j)
                            kr, ki = Z[lz, 2, m:m + 16], Z[lz, 3, m:m + 16]
                            p = (ur * kr - ui * ki, ur * ki + ui * kr)
                            y[i] = p if i not in y else (y[i][0] + p[0], y[i][1] + p[1])
                        yield 16 * (i0 + 2 - max(i0, j))
                    for i in (i0, i0 + 1):
                        Y[l, 0, 16 * i:16 * i + 16, :] = y[i][0].astype(bf16)
                        Y[l, 1, 16 * i:16 * i + 16, :] = y[i][1].astype(bf16)
        return CG * 136 * 16, g()

    def conv_inv(c):
        def g():
            for l in range(CG):
                rg = c * CG + l
                lhs = jnp.concatenate([_packed(Y, (l, part_, slice(0, 8 * NTILE))) for part_ in range(2)], axis=1)
                y = jnp.dot(lhs, _packed(inv_v, (zero[l],)), preferred_element_type=f32)
                for i in range(NTILE):
                    cols = slice(i * T, (i + 1) * T)
                    ga[rg, :, cols] = y[16 * i:16 * i + 16] * (q_v[rg, :, cols].astype(f32) * _rows(gate[0, :, cols], 16))
                yield 512 / 3
        return CG * 512 / 3, g()

    def final16(g_, r16):
        cols = [slice((4 * g_ + a) * T, (4 * g_ + a + 1) * T) for a in range(4)]
        w = [gate[1, :, cols[a]] for a in range(4)]
        for half in (0, 8):
            r = r16 * 16 + half
            rows = slice(r, r + 8) if isinstance(r, int) else pl.ds(pl.multiple_of(r, 8), 8)
            h = yield from recombine8(lambda i: acc[g_, i, rows, :])
            for dq in range(4):
                for a in range(4):
                    idx = (9 * dq + r16, slice(half, half + 8), cols[a])
                    o_v[idx] = (ga[idx] + w[a] * h[dq][a]).astype(bf16)
                yield 12

    def final(g_):
        def g():
            for r16 in range(9):
                yield from final16(g_, r16)
        return 18 * (7 * weight["recombine"] + 48), g()

    def out_copy(g_):
        cols = pl.ds(g_ * 4 * T, 4 * T)
        return pltpu.make_async_copy(o_v.at[:, :, cols], out_hbm.at[:, :, cols], out_sems.at[g_])

    def band_copy(n, dq):
        rows, cols = pl.ds(9 * dq + 3 * n, 3), pl.ds((NTG - 1) * 4 * T, 4 * T)
        return pltpu.make_async_copy(o_v.at[rows, :, cols], out_hbm.at[rows, :, cols], band_sems.at[n, dq])

    def weave(name, matmuls, vector):
        lo, hi, *w = PLAN[name]
        weight.update(zip(("recombine", "gelu", "comb", "load"), w))
        _interleave(_chain(*matmuls()), _chain(*vector()), lo, hi)

    def block(name, matmuls, vector):
        @pl.when(zs[15] == 0)
        def _():
            load_zeros()
            weave(name, matmuls, vector)

    def loop(n, piece):
        def body(i, carry):
            _run((0, piece(i)))
            return carry
        lax.fori_loop(0, n, body, 0)

    def tiles(fn, g_):
        return _chain(*[fn(4 * g_ + a) for a in range(4)])

    def w3_pieces(t, lo, hi):
        return wcomb3([(t, t % 2, n // 8, n % 8) for n in range(lo, hi)])

    def w4_pieces(t, lo, hi):
        return wcomb4([(t, t % 2, n // 9, n % 9) for n in range(lo, hi)])

    load_zeros()
    wait("gw", "sk", "d")
    set_coefs()
    loop(2, acc_zero)
    wait("w1")
    _run(transpose_w(w1_v, w1t))
    loop(1, lambda i: acc_zero(i + 2))
    wait("q0")
    loop(4, lambda c: ln1(c)[1])
    loop(1, lambda i: acc_zero(i + 3))
    wait("q1")
    block("s1", lambda: [tiles(mix1, 0)], lambda: [tiles(ln1, 1)])
    wait("q2", "w2")
    block("s2", lambda: [tiles(mix1, 1)], lambda: [transpose_w(w2_v, w2t), tiles(ln1, 2)])
    wait("q3", *w3_a)
    block("s3", lambda: [tiles(mix1, 2), tiles(mix2, 0)],
          lambda: [w3_pieces(0, 0, 16), wrest(0, 0, 1), wrest(0, 0, 0), tiles(ln1, 3)])
    wait("k0", "v0", *w3_b)
    block("s4", lambda: [tiles(mix1, 3), tiles(mix2, 1)],
          lambda: [acc_init(0), conv_kv(0), conv_kv(1), tiles(ln2, 0), w3_pieces(0, 16, 24), wrest(0, 0, 2)])
    wait("w4_0", "f0", "fwd", "inv")
    start(*later)
    block("s5", lambda: [tiles(mix2, 2), conv_fwd(0, 0)],
          lambda: [acc_init(1), xcomb(0), w4_pieces(0, 0, 10), tiles(ln2, 1)])
    wait("w3_1")
    block("s6", lambda: [tiles(mix2, 3), conv_fwd(1, 1)],
          lambda: [w4_pieces(0, 10, 13), xcomb(1), conv_kv(2), acc_init(2), w3_pieces(1, 0, 6), tiles(ln2, 2)])
    block("s7", lambda: [mm1(0, 0, 0)],
          lambda: [w4_pieces(0, 13, 21), acc_init(3), xcomb(2), conv_bins(0), tiles(ln2, 3), xcomb(3)])

    def stage_a(s, par):
        t, j = (s + 2) // NTG, (s + 2) % NTG
        pieces = []
        for n in range(7):
            n = jnp.minimum(j * 7 + n, 26)
            pieces.append((jnp.minimum(t, NFC - 1), t % 2, n // 9, n % 9))
        weave("a", lambda: [conv_inv(s - 1), mm1(par, s // NTG, s % NTG), conv_fwd(jnp.minimum(s + 1, NU - 1), 1 - par)],
              lambda: [act(1 - par, B), wcomb4(pieces)])

    def stage_b(s):
        t, j = s // NTG + 1, s % NTG
        pieces = []
        for n in range(6):
            n = j * 6 + n
            pieces.append((jnp.minimum(t, NFC - 1), t % 2, n // 8, n % 8))
        weave("b", lambda: [mm2(((s - 1) // NTG) % 2, (s - 1) % NTG, B)],
              lambda: [wrest(jnp.minimum(t, NFC - 1), t % 2, jnp.maximum(j - 1, 0)), wcomb3(pieces), conv_bins(s % 2),
                       conv_kv(jnp.minimum(s + 2, NU - 1))])

    def stage(s, carry):
        pl.when(s == 2)(lambda: wait(*later))
        for par in range(2):
            load_zeros()
            pl.when(s % 2 == par)(lambda: stage_a(s, par))
        pl.when(s < NU - 1)(lambda: stage_b(s))
        return carry

    lax.fori_loop(1, NU, stage, 0)

    par, slot, last = (NU - 1) % 2, (NFC - 1) % 2, NTG - 1
    block("e1", lambda: [mm2(slot, last - 1, B)], lambda: [act(par, B2)])
    block("e2", lambda: [mm2(slot + zero[0], last + zero[0], B2, 0, LAST_CUTS[0])], lambda: [conv_bins(par)])
    for g_ in range(last):
        block("f%d" % g_,
              lambda: ([conv_inv(NU - 1)] if g_ == 0 else []) + [mm2(slot + zero[0], last, B2, LAST_CUTS[g_], LAST_CUTS[g_ + 1])],
              lambda: [final(g_)])
        out_copy(g_).start()
    block("f2", lambda: [mm2(slot + zero[0], last, B2, LAST_CUTS[3], 49)], lambda: [])

    def tail(n, carry):
        for r in range(3):
            _run((0, final16(last, 3 * n + r)))
        for dq in range(4):
            band_copy(n, dq).start()
        return carry

    lax.fori_loop(0, 3, tail, 0)
    for g_ in range(last):
        out_copy(g_).wait()
    for n in range(3):
        for dq in range(4):
            band_copy(n, dq).wait()


@jax.jit
def pallas_gated_mix__ssm_conv_h3__mixer_s_mlp__prompt_kernel(
    A_q: jax.Array,
    A_k: jax.Array,
    A_v: jax.Array,
    A_shift_k: jax.Array,
    A_ssm_k: jax.Array,
    A_ssm_D: jax.Array,
    B_x: jax.Array,
    B_w1: jax.Array,
    B_w2: jax.Array,
    B_w3: jax.Array,
    B_w4: jax.Array,
    gate_w: jax.Array,
):
    del B_x
    fwd, inv = _dft_matrices()
    hbm = pl.BlockSpec(memory_space=pl.ANY)
    vmem = pltpu.VMEM
    scratch = [
        vmem((RG, 16, S), bf16), vmem((RG, 16, S), bf16), vmem((RG, 16, S), bf16), vmem((RG, 16, S), bf16),
        vmem((D, D), bf16), vmem((D, D), bf16), vmem((RG, 16, F), bf16), vmem((RG, 16, F), bf16),
        vmem((4, D), bf16), vmem((D,), bf16), vmem((D,), bf16), vmem((2, T, T), bf16), vmem((1, 2 * T, T), bf16),
        vmem((5, D, T), bf16), vmem((5, D, T), bf16),
        vmem((6, RG, 16, T), f32), vmem((16, T), f32), vmem((2, 8, S), f32),
        vmem((4, D, T), bf16), vmem((4, D, T), bf16),
        vmem((NTILE + 2, D, T), bf16),
        vmem((4, D, T), f32), vmem((4, D, T), f32), vmem((4, D, T), f32), vmem((4, D, T), f32),
        vmem((8, 4, T, T), f32),
        vmem((NTG, 49, 8, 16, T), bf16), vmem((NTG, 4, T, T), bf16),
        vmem((2, KT, 9, 4, 16, T), bf16),
        vmem((2, 49, KT, 10, 16, T), bf16), vmem((2, 49, KT, 9, 16, T), bf16),
        vmem((49, KT, T + 24, T), f32), vmem((49, KT, T + 24, T), f32),
        vmem((49, KT, T, T), bf16), vmem((49, KT, T, T), bf16),
        vmem((NTG, 49, DQ + 16, T), f32),
        vmem((2, CG, 16 * NTILE, T), bf16),
        vmem((2 * CG, 4, 16 * NTILE + 16, T), f32),
        vmem((CG, 2, 16 * NTILE + 32, T), bf16),
        vmem((RG, 16, S), f32), vmem((RG, 16, S), bf16),
        pltpu.SMEM((16,), jnp.int32),
        pltpu.SemaphoreType.DMA((30,)), pltpu.SemaphoreType.DMA((NTG - 1,)), pltpu.SemaphoreType.DMA((3, 4)),
    ]
    out = pl.pallas_call(
        _kernel,
        out_shape=jax.ShapeDtypeStruct((RG, 16, S), bf16),
        in_specs=[hbm] * 13,
        out_specs=hbm,
        scratch_shapes=scratch,
        compiler_params=pltpu.CompilerParams(vmem_limit_bytes=126 * 1024 * 1024),
    )(A_q[0].T.reshape(RG, 16, S), A_k[0].T.reshape(RG, 16, S), A_v[0].T.reshape(RG, 16, S), A_shift_k.T,
      A_ssm_k.reshape(RG, 16, S), A_ssm_D, B_w1, B_w2, B_w3.reshape(RG, 16, F), B_w4.T.reshape(RG, 16, F), gate_w,
      fwd, inv)
    return out.reshape(D, S).T[None]
```

```python
import numpy as np
import ml_dtypes
import jax
import jax.numpy as jnp
from jax import lax
import jax.experimental.pallas as pl
import jax.experimental.pallas.tpu as pltpu

S, D, F = 2048, 576, 4608
T = 128
NTILE = S // T
RG = D // 16
KT = 3
FC = 4 * KT * T
NFC = F // FC
NTG = NTILE // 4
NU = NFC * NTG
CG = RG // NU
DQ = D // 4
DR = D - 4 * T
EPS = 1e-5
GELU_C0 = float(np.sqrt(2.0 / np.pi))
ALPHA = float((0.044715 * GELU_C0) ** (1.0 / 3.0))
f32, bf16, u32 = jnp.float32, jnp.bfloat16, jnp.uint32
SHIFTS = (1, -1, 2, -2)

A_TAB = (((1, 0), (1, 3)), ((1, 2), (1, 3)), ((1, 0),), ((1, 3),), ((1, 0), (1, 1)), ((1, 2), (-1, 0)), ((1, 1), (-1, 3)))
B_TAB = (((1, 0), (1, 3)), ((1, 0),), ((1, 1), (-1, 3)), ((1, 2), (-1, 0)), ((1, 3),), ((1, 0), (1, 1)), ((1, 2), (1, 3)))
C_TAB = (((1, 0), (1, 3)), ((1, 2), (-1, 3)), ((1, 1), (1, 3)), ((1, 0), (1, 2)), ((-1, 0), (1, 1)), ((1, 3),), ((1, 0),))
E_TAB = (None, ((1, 2),), ((1, 1),), None, None, ((1, 3), (-1, 1), (1, 2)), ((1, 0),))
BLANK = [7 * i + j for i in range(7) for j in range(7) if E_TAB[i] is None or E_TAB[j] is None]
R_TAB = (None, (1, 0), None, None, (0, 1), (1, 2), (0, 2))

PLAN = {
    "s1": (0.00, 0.98, 17, 30, 35, 32), "s2": (0.01, 0.98, 11, 30, 34, 32), "s3": (0.00, 1.03, 13, 45, 35, 24),
    "s4": (0.00, 0.97, 11, 31, 43, 25), "s5": (0.00, 1.05, 10, 15, 39, 54), "s6": (0.03, 0.99, 9, 35, 44, 18),
    "s7": (0.08, 1.02, 13, 41, 34, 47), "s8": (0.00, 1.00, 15, 29, 45, 48), "a": (0.04, 0.93, 10, 29, 77, 23),
    "b": (0.02, 0.98, 36, 60, 47, 36), "e1": (0.02, 0.99, 9, 63, 50, 28), "e2": (0.04, 1.00, 13, 30, 47, 32),
    "f0": (0.06, 1.01, 11, 22, 35, 32), "f1": (0.01, 0.96, 13, 41, 18, 32), "f2": (0.01, 0.97, 14, 22, 25, 32),
    "f3": (0.00, 0.97, 13, 22, 25, 32),
}
LAST_CUTS = (18, 20, 31, 42)


def _dft_matrices():
    n = np.arange(T, dtype=np.float64)[:, None]
    f = np.arange(T, dtype=np.float64)[None, :]
    theta = 2.0 * np.pi * (f + 0.5) * n / (2 * T)
    fwd = np.stack([np.cos(theta), -np.sin(theta)])
    inv = np.concatenate([fwd[0].T, fwd[1].T])[None] / T
    return fwd.astype(ml_dtypes.bfloat16), inv.astype(ml_dtypes.bfloat16)


def _comb(tab, quad):
    (_, first), *rest = tab
    v = quad[first]
    for sign, o in rest:
        v = v + quad[o] if sign > 0 else v - quad[o]
    return v


def _blk(o, p):
    return 2 * (o // 2) + p // 2, 2 * (o % 2) + p % 2


def _gelu(h):
    return h * (1.0 + jnp.tanh(h * (GELU_C0 / ALPHA + h * h)))


def _chain(*streams):
    def g():
        for s in streams:
            yield from s[1]
    return sum(s[0] for s in streams), g()


def _run(*streams):
    for s in streams:
        for _ in s[1]:
            pass


def _interleave(first, second, lo, hi):
    live = [[0.0, float(first[0]) or 1.0, first[1], 0.0, 1.0], [0.0, float(second[0]) or 1.0, second[1], lo, hi]]
    while live:
        live.sort(key=lambda x: x[3] + (x[4] - x[3]) * x[0] / x[1])
        try:
            live[0][0] += next(live[0][2])
        except StopIteration:
            live.pop(0)


def _packed(ref, idx):
    v = ref.bitcast(u32)[idx]
    if v.ndim == 3:
        v = v.reshape(v.shape[0] * v.shape[1], v.shape[2])
    return pltpu.bitcast(v, bf16)


def _vsum(x):
    parts = [x[r:r + 8] for r in range(0, x.shape[0], 8)]
    while len(parts) > 1:
        parts = [parts[i] + parts[i + 1] for i in range(0, len(parts) - 1, 2)] + ([parts[-1]] if len(parts) % 2 else [])
    return parts[0]


def _rows(stat, n):
    return jnp.concatenate([stat] * (n // 8), axis=0)


def _kernel(q_hbm, k_hbm, v_hbm, sk_hbm, f_hbm, d_hbm, w1_hbm, w2_hbm, w3_hbm, w4_hbm, gw_hbm, fwd_hbm, inv_hbm,
            out_hbm,
            q_v, k_v, v_v, f_v, w1_v, w2_v, w3_v, w4_v, sk_v, d_v, gw_v, fwd_v, inv_v,
            w1t, w2t, coef, sign, gate, xn0, xn1, HR, x1a, x1b, x1c, x1d, XT, XS, XE, WR, W3C, W4C, p0, p1, B, B2, acc,
            KV, Z, Y, ga, o_v, zs, in_sems, out_sems):
    XN, X1, P = (xn0, xn1), (x1a, x1b, x1c, x1d), (p0, p1)
    every = slice(None)
    weight = {}
    zero = []

    pairs = dict(gw=(gw_hbm, gw_v), sk=(sk_hbm, sk_v), d=(d_hbm, d_v), w1=(w1_hbm, w1_v), w2=(w2_hbm, w2_v),
                 fwd=(fwd_hbm, fwd_v), inv=(inv_hbm, inv_v))

    def part(name, src, dst, idx):
        pairs[name] = (src.at[idx], dst.at[idx])

    for g_ in range(NTG):
        part("q%d" % g_, q_hbm, q_v, (every, every, pl.ds(g_ * 4 * T, 4 * T)))
    for name, src, dst, first in (("k", k_hbm, k_v, 4 * CG), ("v", v_hbm, v_v, 4 * CG), ("f", f_hbm, f_v, 3 * CG)):
        part(name + "0", src, dst, pl.ds(0, first))
        part(name, src, dst, pl.ds(first, RG - first))
    for fq in range(4):
        part("w3_a%d" % fq, w3_hbm, w3_v, (every, every, pl.ds(fq * KT * T, 2 * T)))
        part("w3_b%d" % fq, w3_hbm, w3_v, (every, every, pl.ds(fq * KT * T + 2 * T, T)))
    for t in range(NFC):
        if t:
            part("w3_%d" % t, w3_hbm, w3_v, (every, every, pl.ds(t * FC, FC)))
        part("w4_%d" % t, w4_hbm, w4_v, (every, every, pl.ds(t * FC, FC)))
    w3_a, w3_b = ["w3_a%d" % fq for fq in range(4)], ["w3_b%d" % fq for fq in range(4)]
    early = ["gw", "sk", "d", "w1", "q0", "q1", "w2", "q2", "q3"] + w3_a + ["k0", "v0"] + w3_b \
        + ["w4_0", "f0", "fwd", "inv", "w3_1"]
    later = ["w4_1", "f", "k", "v", "w3_2", "w4_2"]
    copies = {n: pltpu.make_async_copy(pairs[n][0], pairs[n][1], in_sems.at[i]) for i, n in enumerate(early + later)}

    def start(*names):
        for n in names:
            copies[n].start()

    def wait(*names):
        for n in names:
            copies[n].wait()

    start(*early, *later)
    for i in range(16):
        zs[i] = 0
    HR[0] = jnp.zeros((D, T), bf16)
    HR[NTILE + 1] = jnp.zeros((D, T), bf16)
    lane16 = lax.broadcasted_iota(jnp.int32, (16, T), 1)
    lane72 = lax.broadcasted_iota(jnp.int32, (DQ // 2, T), 1)
    sign[...] = (1 - 2 * (lane16 & 1)).astype(f32)

    def load_zeros():
        zero[:] = [zs[i] for i in range(16)]

    def combos16(tab, blk, store):
        for i in (6, 4, 1, 3, 0, 5, 2):
            inner = [_comb(tab[i], [blk[_blk(o, p)[0]][_blk(o, p)[1]] for o in range(4)]) for p in range(4)]
            for j in range(7):
                store(7 * i + j, _comb(tab[j], inner).astype(bf16))
            yield weight["comb"]

    def recombine8(load, quadrants=(0, 1, 2, 3)):
        h = [[None] * 4 for _ in range(4)]
        for i in (4, 1, 2, 0, 3, 5, 6):
            targets = [(s, o) for s, o in C_TAB[i] if o in quadrants]
            if not targets:
                continue
            m = [load(7 * i + j) for j in range(7)]
            quad = [m[0] + m[3] - m[4] + m[6], m[2] + m[4], m[1] + m[3], m[0] - m[1] + m[2] + m[5]]
            for s, o in targets:
                for p in range(4):
                    a, b = _blk(o, p)
                    if h[a][b] is None:
                        h[a][b] = quad[p] if s > 0 else -quad[p]
                    else:
                        h[a][b] = h[a][b] + quad[p] if s > 0 else h[a][b] - quad[p]
            yield weight["recombine"]
        return h

    def transpose_w(src, dst):
        def g():
            for kt in range(5):
                n = T if kt < 4 else DR
                w = src[kt * T:kt * T + n, :].astype(f32)
                if n < T:
                    w = jnp.concatenate([w, jnp.zeros((T - n, D), f32)], axis=0)
                dst[kt] = w.T.astype(bf16)
                yield 100
        return 500, g()

    def coefs(*which):
        def g():
            for i in which:
                if i < 4:
                    row = sk_v[...].astype(f32)[i:i + 1]
                else:
                    row = (d_v if i == 4 else gw_v)[...].astype(f32).reshape(1, D)
                coef[i] = jnp.broadcast_to(row, (T, D)).T.reshape(RG, 16, T)
                yield 80
        return 80 * len(which), g()

    def centred_scale(xg, a, total, z):
        mean = jnp.broadcast_to(jnp.sum(total, axis=0, keepdims=True) * (1.0 / D), (8, T))
        sq = None
        for r in range(0, D, 64):
            x = xg[a + z, r:r + 64, :] - _rows(mean, 64)
            part_sq = _vsum(x * x)
            sq = part_sq if sq is None else sq + part_sq
            yield 24
        var = jnp.sum(sq, axis=0, keepdims=True) * (1.0 / D)
        return mean, jnp.broadcast_to(ALPHA * lax.rsqrt(var + (2.0 * ALPHA) ** 2 * EPS), (8, T))

    def ln1(c):
        if isinstance(c, int):
            cols, xn, xg, a = slice(c * T, (c + 1) * T), XN[(c // 4) % 2], X1[c // 4], c % 4
        else:
            cols, xn, xg, a = pl.ds(pl.multiple_of(c * T, T), T), XN[0], X1[0], c

        def g():
            total = logit = None
            for r in range(0, RG, 4):
                x = q_v[r:r + 4, :, cols].astype(f32).reshape(64, T) * (2.0 * ALPHA)
                xg[a, 16 * r:16 * r + 64, :] = x
                s, l = _vsum(x), _vsum(x * coef[5, r:r + 4].reshape(64, T))
                total = s if total is None else total + s
                logit = l if logit is None else logit + l
                yield 40
            g_val = jax.nn.sigmoid(jnp.sum(logit, axis=0, keepdims=True) * (0.5 / ALPHA))
            gate[0, :, cols] = jnp.broadcast_to(g_val, (8, T))
            gate[1, :, cols] = jnp.broadcast_to((1.0 - g_val) * (0.5 / ALPHA), (8, T))
            mean, scale = yield from centred_scale(xg, a, total, zero[0])
            for r in range(0, D, 64):
                xn[a, r:r + 64, :] = ((xg[a + zero[1], r:r + 64, :] - _rows(mean, 64)) * _rows(scale, 64)).astype(bf16)
                yield 20
        return 9 * 84, g()

    def lhs_w(wt, rows):
        r2 = slice(rows.start // 2, rows.stop // 2)
        return jnp.concatenate([_packed(wt, (kt, r2)) for kt in range(4)] + [_packed(wt, (4, r2))[:, :DR]], axis=1)

    def mix1(c):
        def g():
            for qi, sh in enumerate(SHIFTS):
                rows = slice(qi * DQ, (qi + 1) * DQ)
                h = jnp.dot(lhs_w(w1t, rows), _packed(XN[(c // 4) % 2], (c % 4 + zero[2 + qi],)), preferred_element_type=f32)
                HR[c + 1, rows, :] = _gelu(pltpu.roll(h, sh % T, 1)).astype(bf16)
                yield 5 * DQ / 3
        return 5 * D / 3, g()

    def mix2(c):
        def g():
            hv = HR.bitcast(u32)
            parts = []
            for qi, sh in enumerate(SHIFTS):
                r2 = slice(qi * DQ // 2, (qi + 1) * DQ // 2)
                own, neighbour = hv[c + 1, r2, :], hv[c if sh > 0 else c + 2, r2, :]
                parts.append(jnp.where(lane72 >= sh if sh > 0 else lane72 < T + sh, own, neighbour))
            rhs = pltpu.bitcast(jnp.concatenate(parts, axis=0), bf16)
            for qi in range(4):
                rows = slice(qi * DQ, (qi + 1) * DQ)
                X1[c // 4][c % 4, rows, :] += jnp.dot(lhs_w(w2t, rows), rhs, preferred_element_type=f32)
                yield 5 * DQ / 3
        return 5 * D / 3, g()

    def ln2(c):
        xg, a = X1[c // 4], c % 4

        def g():
            total = None
            for r in range(0, D, 96):
                s = _vsum(xg[a, r:r + 96, :])
                total = s if total is None else total + s
                yield 12
            mean, scale = yield from centred_scale(xg, a, total, zero[6])
            for kt in range(5):
                n = T if kt < 4 else DR
                x = (xg[a + zero[7], kt * T:kt * T + n, :] - _rows(mean, n)) * _rows(scale, n)
                if n < T:
                    XE[c // 4, a] = jnp.concatenate([x, jnp.zeros((T - n, T), f32)], axis=0).T.astype(bf16)
                else:
                    XT[c % 8, kt] = x.T
                yield 40
        return 72 + 216 + 200, g()

    def xcomb(g_):
        def g():
            for r in range(0, T, 16):
                blk = [[XT[(4 * g_ + a) % 8, kt, r:r + 16, :] for kt in range(4)] for a in range(4)]

                def store(i, val):
                    XS[g_, i, r // 16] = val
                yield from combos16(A_TAB, blk, store)
        return 8 * 7 * weight["comb"], g()

    def acc_zero(g_):
        for i in BLANK:
            acc[g_, i, 0:DQ] = jnp.zeros((DQ, T), f32)
        yield 0

    def acc_init(g_):
        def g():
            for r in range(0, DQ, 24):
                blk = [[X1[g_][a, dq * DQ + r:dq * DQ + r + 24, :] for a in range(4)] for dq in range(4)]
                for i in range(7):
                    if E_TAB[i] is not None:
                        inner = [_comb(E_TAB[i], [blk[_blk(o, p)[0]][_blk(o, p)[1]] for o in range(4)]) for p in range(4)]
                        for j in range(7):
                            if E_TAB[j] is not None:
                                acc[g_, 7 * i + j, r:r + 24, :] = _comb(E_TAB[j], inner)
                        yield 24
        return 6 * 4 * 24, g()

    def feature_tile(t, fq, kt):
        return pl.ds(pl.multiple_of(t * FC + KT * T * fq + T * kt, T), T)

    def wcomb3(pieces):
        def g():
            for t, slot, kt, r in pieces:
                blk = [[w3_v[8 * k + r, :, feature_tile(t, fq, kt)].astype(f32) for fq in range(4)] for k in range(4)]
                yield weight["load"]

                def store(i, val):
                    W3C[slot, i, kt, r] = val
                yield from combos16(B_TAB, blk, store)
        return len(pieces) * (weight["load"] + 7 * weight["comb"]), g()

    def wrest(t, slot, kt):
        def g():
            for r in range(4):
                w = [w3_v[32 + r, :, feature_tile(t, fq, kt)].astype(f32) for fq in range(4)]
                for c1, row in enumerate(((w[0], w[1]), (w[2], w[3]), (w[0] + w[2], w[1] + w[3]))):
                    for c2, val in enumerate((row[0], row[1], row[0] + row[1])):
                        WR[slot, kt, 3 * c1 + c2, r] = val.astype(bf16)
                yield 30
        return 120, g()

    def wcomb4(pieces):
        def g():
            for t, slot, kt, r in pieces:
                blk = [[w4_v[9 * dq + r, :, feature_tile(t, fq, kt)].astype(f32) for fq in range(4)] for dq in range(4)]
                yield weight["load"]

                def store(i, val):
                    W4C[slot, i, kt, r] = val
                yield from combos16(A_TAB, blk, store)
        return len(pieces) * (weight["load"] + 7 * weight["comb"]), g()

    def mm1(par, t, g_, kts=(0, 1, 2)):
        def g():
            for kt in kts:
                for i in range(49):
                    m = jnp.dot(_packed(XS, (g_, i, slice(0, 8))), _packed(W3C, (t % 2, i, kt, slice(0, 8))),
                                preferred_element_type=f32)
                    r1, r2 = R_TAB[i // 7], R_TAB[i % 7]
                    rest = r1 is not None and r2 is not None
                    if rest:
                        m = m + jnp.dot(_packed(XE, (g_, 2 * r1[0] + r2[0]))[:, :DR], _packed(WR, (t % 2, kt, 3 * r1[1] + r2[1])),
                                        preferred_element_type=f32)
                    P[par][i, kt, 0:T] = m
                    yield T * (1 + rest) / KT
        return 65 * T * len(kts) / KT, g()

    def gelu8(par, kt, r):
        h = yield from recombine8(lambda i: P[par][i, kt, r:r + 8, :])
        for o in range(4):
            for p in range(4):
                a, fq = _blk(o, p)
                h[a][fq] = _gelu(h[a][fq])
            yield weight["gelu"]
        return h

    def act(par, dst):
        def g():
            for kt in range(KT):
                for r in range(0, T, 16):
                    h0 = yield from gelu8(par, kt, r)
                    h1 = yield from gelu8(par, kt, r + 8)
                    blk = [[jnp.concatenate([h0[a][fq], h1[a][fq]], axis=0) for a in range(4)] for fq in range(4)]

                    def store(i, val):
                        dst[i, kt, r:r + 16, :] = val
                    yield from combos16(B_TAB, blk, store)
        return 24 * (2 * (7 * weight["recombine"] + 4 * weight["gelu"]) + 7 * weight["comb"]), g()

    def mm2(slot, g_, src, products=range(49)):
        def g():
            for i in products:
                lhs = jnp.concatenate([_packed(W4C, (slot, i, kt)) for kt in range(KT)], axis=1)
                rhs = jnp.concatenate([_packed(src, (i, kt)) for kt in range(KT)], axis=1)
                acc[g_, i, 0:DQ] += lax.dot_general(lhs, rhs, (((1,), (1,)), ((), ())), preferred_element_type=f32)
                yield DQ
        return len(products) * DQ, g()

    def conv_kv(c):
        def g():
            for l in range(CG):
                rg = c * CG + l
                cf = [coef[j, rg] for j in range(4)]
                prev = None
                for tt in range(NTILE):
                    cols = slice(tt * T, (tt + 1) * T)
                    kk = k_v[rg, :, cols].astype(f32)
                    rolled = [pltpu.roll(kk * cf[j], j, 1) for j in (1, 2, 3)]
                    ks = kk * cf[0]
                    for j in (1, 2, 3):
                        ks = ks + jnp.where(lane16 >= j, rolled[j - 1], 0.0 if prev is None else prev[j - 1])
                    prev = rolled
                    KV[c % 2, l, tt * 16:(tt + 1) * 16, :] = (ks * v_v[rg, :, cols].astype(f32)).astype(bf16)
                    yield 27
        return CG * NTILE * 27, g()

    def conv_fwd(c, par):
        def g():
            def dft(z):
                return jnp.concatenate([_packed(fwd_v, (z,)), _packed(fwd_v, (z + 1,))], axis=1)
            for l in range(CG):
                rg, lz = c * CG + l, par * CG + l
                z = jnp.dot(_packed(KV, (par, l)), dft(zero[2 * l]), preferred_element_type=f32)
                Z[lz, 0, 0:16 * NTILE] = z[:, :T]
                Z[lz, 1, 0:16 * NTILE] = z[:, T:]
                yield 512 / 3
                taps = jnp.concatenate([f_v[rg, :, m * T:(m + 1) * T] for m in range(NTILE)], axis=0)
                z = jnp.dot(taps, dft(zero[2 * l + 1]), preferred_element_type=f32)
                for m in range(NTILE):
                    kr, ki = z[16 * m:16 * m + 16, :T], z[16 * m:16 * m + 16, T:]
                    if m == 0:
                        kr = kr + coef[4, rg]
                    else:
                        sigma = sign[...]
                        kr = kr - sigma * z[16 * m - 16:16 * m, T:]
                        ki = ki + sigma * z[16 * m - 16:16 * m, :T]
                    Z[lz, 2, 16 * m:16 * m + 16] = kr
                    Z[lz, 3, 16 * m:16 * m + 16] = ki
                yield 512 / 3
        return CG * 1024 / 3, g()

    def conv_bins(par):
        def g():
            for i0 in range(NTILE - 2, -1, -2):
                for l in range(CG):
                    lz = par * CG + l + zero[i0 // 2]
                    y = {}
                    for j in range(i0 + 2):
                        ur, ui = Z[lz, 0, 16 * j:16 * j + 16], Z[lz, 1, 16 * j:16 * j + 16]
                        for i in range(max(i0, j), i0 + 2):
                            m = 16 * (i - j)
                            kr, ki = Z[lz, 2, m:m + 16], Z[lz, 3, m:m + 16]
                            p = (ur * kr - ui * ki, ur * ki + ui * kr)
                            y[i] = p if i not in y else (y[i][0] + p[0], y[i][1] + p[1])
                        yield 16 * (i0 + 2 - max(i0, j))
                    for i in (i0, i0 + 1):
                        Y[l, 0, 16 * i:16 * i + 16, :] = y[i][0].astype(bf16)
                        Y[l, 1, 16 * i:16 * i + 16, :] = y[i][1].astype(bf16)
        return CG * 136 * 16, g()

    def conv_inv(c):
        def g():
            for l in range(CG):
                rg = c * CG + l
                lhs = jnp.concatenate([_packed(Y, (l, part_, slice(0, 8 * NTILE))) for part_ in range(2)], axis=1)
                y = jnp.dot(lhs, _packed(inv_v, (zero[l],)), preferred_element_type=f32)
                for i in range(NTILE):
                    cols = slice(i * T, (i + 1) * T)
                    ga[rg, :, cols] = y[16 * i:16 * i + 16] * (q_v[rg, :, cols].astype(f32) * _rows(gate[0, :, cols], 16))
                yield 512 / 3
        return CG * 512 / 3, g()

    def final16(g_, r16, quadrants):
        cols = [slice((4 * g_ + a) * T, (4 * g_ + a + 1) * T) for a in range(4)]
        for half in (0, 8):
            r = r16 * 16 + half
            rows = slice(r, r + 8) if isinstance(r, int) else pl.ds(pl.multiple_of(r, 8), 8)
            h = yield from recombine8(lambda i: acc[g_, i, rows, :], quadrants)
            for dq in range(4):
                for a in range(4):
                    if h[dq][a] is not None:
                        idx = (9 * dq + r16, slice(half, half + 8), cols[a])
                        o_v[idx] = (ga[idx] + gate[1, :, cols[a]] * h[dq][a]).astype(bf16)
                yield 3 * len(quadrants)

    def final(g_, quadrants=(0, 1, 2, 3)):
        def g():
            for r16 in range(9):
                yield from final16(g_, r16, quadrants)
        return 18 * (7 * weight["recombine"] + 12 * len(quadrants)), g()

    half_rows, last_col = RG // 2, (NTG - 1) * 4 * T
    out_parts = [(every, every, pl.ds(g_ * 4 * T, 4 * T)) for g_ in range(NTG - 1)] + [
        (pl.ds(0, half_rows), every, pl.ds(last_col, 4 * T)),
        (pl.ds(half_rows, half_rows), every, pl.ds(last_col, 2 * T)),
        (pl.ds(half_rows, half_rows), every, pl.ds(last_col + 2 * T, 2 * T))]
    out_copies = [pltpu.make_async_copy(o_v.at[idx], out_hbm.at[idx], out_sems.at[n]) for n, idx in enumerate(out_parts)]

    def weave(name, matmuls, vector):
        lo, hi, *w = PLAN[name]
        weight.update(zip(("recombine", "gelu", "comb", "load"), w))
        _interleave(_chain(*matmuls()), _chain(*vector()), lo, hi)

    def block(name, matmuls, vector):
        @pl.when(zs[15] == 0)
        def _():
            load_zeros()
            weave(name, matmuls, vector)

    def loop(n, piece):
        def body(i, carry):
            _run((0, piece(i)))
            return carry
        lax.fori_loop(0, n, body, 0)

    def tiles(fn, g_):
        return _chain(*[fn(4 * g_ + a) for a in range(4)])

    def w3_pieces(lo, hi):
        return wcomb3([(0, 0, n // 8, n % 8) for n in range(lo, hi)])

    def w4_pieces(lo, hi):
        return wcomb4([(0, 0, n // 9, n % 9) for n in range(lo, hi)])

    load_zeros()
    wait("gw", "sk", "d")
    _run(coefs(5))
    loop(3, acc_zero)
    wait("w1")
    _run(transpose_w(w1_v, w1t))
    loop(1, lambda i: acc_zero(i + 3))
    wait("q0")
    loop(4, lambda c: ln1(c)[1])
    wait("q1")
    block("s1", lambda: [tiles(mix1, 0)], lambda: [tiles(ln1, 1)])
    wait("q2", "w2")
    block("s2", lambda: [tiles(mix1, 1)], lambda: [transpose_w(w2_v, w2t), tiles(ln1, 2)])
    wait("q3", *w3_a)
    block("s3", lambda: [tiles(mix1, 2), tiles(mix2, 0)],
          lambda: [tiles(ln1, 3), wrest(0, 0, 0), wrest(0, 0, 1), w3_pieces(0, 16), coefs(0, 1, 2, 3, 4)])
    wait("k0", "v0", *w3_b)
    block("s4", lambda: [tiles(mix1, 3), tiles(mix2, 1)],
          lambda: [tiles(ln2, 0), conv_kv(1), wrest(0, 0, 2), conv_kv(0), w3_pieces(16, 24), acc_init(0)])
    wait("w4_0", "f0", "fwd", "inv")
    block("s5", lambda: [tiles(mix2, 2), conv_fwd(0, 0)],
          lambda: [acc_init(1), xcomb(0), w4_pieces(0, 8), tiles(ln2, 1)])
    block("s6", lambda: [tiles(mix2, 3)], lambda: [acc_init(2), xcomb(1), w4_pieces(8, 11), tiles(ln2, 2)])
    block("s7", lambda: [mm1(0, 0, 0, (0,))], lambda: [acc_init(3), xcomb(2), tiles(ln2, 3)])
    block("s8", lambda: [mm1(0, 0, 0, (1, 2))], lambda: [conv_bins(0), xcomb(3), w4_pieces(11, 21)])
    wait("w3_1")

    def stage_a(s, par):
        t, j = (s + 2) // NTG, (s + 2) % NTG
        pieces = []
        for n in range(7):
            n = jnp.minimum(j * 7 + n, 26)
            pieces.append((jnp.minimum(t, NFC - 1), t % 2, n // 9, n % 9))
        weave("a", lambda: [conv_inv(s - 1), mm1(par, s // NTG, s % NTG), conv_fwd(s, par)],
              lambda: [act(1 - par, B), wcomb4(pieces)])

    def stage_b(s):
        t = s // NTG + 1
        target = (jnp.minimum(t, NFC - 1), t % 2, jnp.maximum(s % NTG - 1, 0))
        weave("b", lambda: [mm2(((s - 1) // NTG) % 2, (s - 1) % NTG, B)],
              lambda: [conv_bins(s % 2), wcomb3([target + (r,) for r in range(8)]), wrest(*target), conv_kv(s + 1)])

    def stage(s, carry):
        pl.when(s == 2)(lambda: wait(*later))
        for par in range(2):
            load_zeros()
            pl.when(s % 2 == par)(lambda: stage_a(s, par))
        pl.when(s < NU - 1)(lambda: stage_b(s))
        return carry

    lax.fori_loop(1, NU, stage, 0)

    par, slot, last = (NU - 1) % 2, (NFC - 1) % 2, NTG - 1
    order = [7 * i + j for i in (0, 1, 2, 3, 4, 6, 5) for j in range(7)]
    block("e1", lambda: [mm2(slot, last - 1, B)], lambda: [act(par, B2)])
    block("e2", lambda: [mm2(slot + zero[0], last + zero[0], B2, order[:LAST_CUTS[0]])], lambda: [conv_bins(par)])
    for g_ in range(last):
        block("f%d" % g_,
              lambda: ([conv_inv(NU - 1)] if g_ == 0 else []) + [mm2(slot + zero[0], last, B2, order[LAST_CUTS[g_]:LAST_CUTS[g_ + 1]])],
              lambda: [final(g_)])
        out_copies[g_].start()
    block("f3", lambda: [mm2(slot + zero[0], last, B2, order[LAST_CUTS[3]:])], lambda: [final(last, (0, 1, 2))])
    out_copies[last].start()
    out_copies[last + 1].start()
    loop(9, lambda r16: final16(last, r16, (3,)))
    out_copies[last + 2].start()
    for copy in out_copies:
        copy.wait()


@jax.jit
def pallas_gated_mix__ssm_conv_h3__mixer_s_mlp__prompt_kernel(
    A_q: jax.Array,
    A_k: jax.Array,
    A_v: jax.Array,
    A_shift_k: jax.Array,
    A_ssm_k: jax.Array,
    A_ssm_D: jax.Array,
    B_x: jax.Array,
    B_w1: jax.Array,
    B_w2: jax.Array,
    B_w3: jax.Array,
    B_w4: jax.Array,
    gate_w: jax.Array,
):
    del B_x
    fwd, inv = _dft_matrices()
    hbm = pl.BlockSpec(memory_space=pl.ANY)
    vmem = pltpu.VMEM
    scratch = [
        vmem((RG, 16, S), bf16), vmem((RG, 16, S), bf16), vmem((RG, 16, S), bf16), vmem((RG, 16, S), bf16),
        vmem((D, D), bf16), vmem((D, D), bf16), vmem((RG, 16, F), bf16), vmem((RG, 16, F), bf16),
        vmem((4, D), bf16), vmem((D,), bf16), vmem((D,), bf16), vmem((2, T, T), bf16), vmem((1, 2 * T, T), bf16),
        vmem((5, D, T), bf16), vmem((5, D, T), bf16),
        vmem((6, RG, 16, T), f32), vmem((16, T), f32), vmem((2, 8, S), f32),
        vmem((4, D, T), bf16), vmem((4, D, T), bf16),
        vmem((NTILE + 2, D, T), bf16),
        vmem((4, D, T), f32), vmem((4, D, T), f32), vmem((4, D, T), f32), vmem((4, D, T), f32),
        vmem((8, 4, T, T), f32),
        vmem((NTG, 56, 9, 16, T), bf16), vmem((NTG, 4, T, T), bf16),
        vmem((2, KT, 9, 4, 16, T), bf16),
        vmem((2, 49, KT, 10, 16, T), bf16), vmem((2, 49, KT, 9, 16, T), bf16),
        vmem((49, KT, T + 24, T), f32), vmem((49, KT, T + 24, T), f32),
        vmem((49, KT, T, T), bf16), vmem((49, KT, T, T), bf16),
        vmem((NTG, 52, DQ + 8, T), f32),
        vmem((2, CG, 16 * NTILE, T), bf16),
        vmem((2 * CG, 4, 16 * NTILE + 16, T), f32),
        vmem((CG, 2, 16 * NTILE + 32, T), bf16),
        vmem((RG, 16, S), f32), vmem((RG, 16, S), bf16),
        pltpu.SMEM((16,), jnp.int32),
        pltpu.SemaphoreType.DMA((30,)), pltpu.SemaphoreType.DMA((NTG + 2,)),
    ]
    out = pl.pallas_call(
        _kernel,
        out_shape=jax.ShapeDtypeStruct((RG, 16, S), bf16),
        in_specs=[hbm] * 13,
        out_specs=hbm,
        scratch_shapes=scratch,
        compiler_params=pltpu.CompilerParams(vmem_limit_bytes=126 * 1024 * 1024),
    )(A_q[0].T.reshape(RG, 16, S), A_k[0].T.reshape(RG, 16, S), A_v[0].T.reshape(RG, 16, S), A_shift_k.T,
      A_ssm_k.reshape(RG, 16, S), A_ssm_D, B_w1, B_w2, B_w3.reshape(RG, 16, F), B_w4.T.reshape(RG, 16, F), gate_w,
      fwd, inv)
    return out.reshape(D, S).T[None]
```
